```python
import os as _os
_os.environ.setdefault("JAX_PLATFORMS", "cpu")
import jax
import jax.numpy as jnp

def _softmax(x, axis=-1):
    return jax.nn.softmax(x, axis=axis)
def _gelu(x):
    return jax.nn.gelu(x, approximate=True)
def _silu(x):
    return jax.nn.silu(x)
def _sigmoid(x):
    return jax.nn.sigmoid(x)
def _layernorm(x, axis=-1, eps=1e-5):
    m = jnp.mean(x, axis=axis, keepdims=True)
    v = jnp.var(x, axis=axis, keepdims=True)
    return (x - m) / jnp.sqrt(v + eps)
def _scatter_add(tgt, idx, src, axis=0):
    return tgt.at[idx].add(src)
def _segment_sum(src, seg, n):
    return jax.ops.segment_sum(src, seg, n)
class _Rng:
    def __init__(self, key):
        self._k = key
    def _next(self):
        self._k, sub = jax.random.split(self._k)
        return sub
    def normal(self, shape):
        return jax.random.normal(self._next(), shape, dtype=jnp.bfloat16)
    def randint(self, lo, hi, shape):
        return jax.random.randint(self._next(), shape, lo, hi, dtype=jnp.int32)
    def uniform(self, shape, lo=0.0, hi=1.0):
        return jax.random.uniform(self._next(), shape, jnp.bfloat16, lo, hi)
    def permutation(self, n):
        return jax.random.permutation(self._next(), n)


kernel_name = 'concat_heads__sliding_block__ssm_conv_s4__prompt'

def setup_inputs():
    _rng = _Rng(jax.random.key(int.from_bytes(__import__("os").urandom(4), "little")))
    _w = (lambda a: (lambda t: t.astype(jnp.bfloat16) if jnp.issubdtype(t.dtype, jnp.floating) else t)(jnp.asarray(a)))
    def _A_setup():
        B, S, D = 1, 2048, 512
        return {
            "x": _w((lambda *s: _rng.normal(s) * 0.2)(B, S, D)),
            "wqkv": _w((lambda *s: _rng.normal(s) * 0.2)(D, 3 * D)),
            "wo": _w((lambda *s: _rng.normal(s) * 0.05)(D, D)),
        }
    _A_in = _A_setup()

    def _B_setup():
        B, L, D, N = 1, 2048, 512, 128
        A_re = -jnp.exp((lambda *s: _rng.normal(s) * 0.8)(D, N))
        A_im = jnp.pi * (lambda *s: _rng.normal(s) * 0.8)(D, N)
        B_re = (lambda *s: _rng.normal(s) * 0.8)(D, N)
        B_im = (lambda *s: _rng.normal(s) * 0.8)(D, N)
        C_re = (lambda *s: _rng.normal(s) * 0.8)(D, N)
        C_im = (lambda *s: _rng.normal(s) * 0.8)(D, N)
        log_dt = (lambda *s: _rng.normal(s) * 0.8)(D) * 0.5 - 4.0
        Dskip = (lambda *s: _rng.normal(s) * 0.05)(D)
        return {
            "u": _w((lambda *s: _rng.normal(s) * 0.05)(B, L, D)),
            "A_re": _w(A_re),
            "A_im": _w(A_im),
            "B_re": _w(B_re),
            "B_im": _w(B_im),
            "C_re": _w(C_re),
            "C_im": _w(C_im),
            "log_dt": _w(log_dt),
            "Dskip": _w(Dskip),
        }
    _B_in = _B_setup()

    return {
        "A_x": _A_in["x"],
        "A_wqkv": _A_in["wqkv"],
        "A_wo": _A_in["wo"],
        "B_u": _B_in["u"],
        "B_A_re": _B_in["A_re"],
        "B_A_im": _B_in["A_im"],
        "B_B_re": _B_in["B_re"],
        "B_B_im": _B_in["B_im"],
        "B_C_re": _B_in["C_re"],
        "B_C_im": _B_in["C_im"],
        "B_log_dt": _B_in["log_dt"],
        "B_Dskip": _B_in["Dskip"],
    }

def reference(A_x, A_wqkv, A_wo, B_u, B_A_re, B_A_im, B_B_re, B_B_im, B_C_re, B_C_im, B_log_dt, B_Dskip):
    def _A_ref(x, wqkv, wo):
        B, S, D = x.shape
        H = 32; Dh = D // H; W = 256
        qkv = (lambda x, *d: x.transpose(*d))((x @ wqkv).reshape(B, S, 3, H, Dh), 2, 0, 3, 1, 4)
        q, k, v = qkv[0], qkv[1], qkv[2]
        scores = jnp.einsum("bhqd,bhkd->bhqk", q, k) * (Dh ** -0.5)
        idx = jnp.arange(S)
        mask = (idx[:, None] - idx[None, :] >= 0) & (idx[:, None] - idx[None, :] < W)
        scores = jnp.where(mask[None, None], scores, -1e9)
        p = _softmax(scores, axis=-1)
        o = jnp.einsum("bhqk,bhkd->bhqd", p, v)
        return (lambda x, *d: x.transpose(*d))(o, 0, 2, 1, 3).reshape(B, S, D) @ wo

    def _B_ref(u, A_re, A_im, B_re, B_im, C_re, C_im, log_dt, Dskip):
        Bsz, L, D = u.shape
        dt = jnp.exp(log_dt)[:, None]
        A = A_re + 1j * A_im
        Bc = B_re + 1j * B_im
        Cc = C_re + 1j * C_im
        logdA = dt * A
        dB = dt * Bc
        l = (lambda x, dt: x.astype(dt))(jnp.arange(L), A_re.dtype)
        P = jnp.exp(logdA[:, :, None] * l[None, None, :])
        K = jnp.einsum("dn,dnl,dn->dl", Cc, P, dB).real
        L2 = 2 * L
        Kp = jnp.pad(K, ((0, 0), (0, L)))
        up = (lambda x, *d: x.transpose(*d))(u, 0, 2, 1)
        up = jnp.pad(up, ((0, 0), (0, 0), (0, L)))
        Kf = (lambda x, axes=(-2,-1): jnp.fft.rfft2(x.astype(jnp.float32), axes=axes))(Kp[:, None, :], axes=(-2, -1))
        Uf = (lambda x, axes=(-2,-1): jnp.fft.rfft2(x.astype(jnp.float32), axes=axes))(up[:, :, None, :], axes=(-2, -1))
        Yf = Uf * Kf[None, :, :, :]
        y = (lambda x, s, axes=(-2,-1): jnp.fft.irfft2(x, s=s, axes=axes).astype(jnp.bfloat16))(Yf, (1, L2), axes=(-2, -1))[:, :, 0, :L]
        y = (lambda x, *d: x.transpose(*d))(y, 0, 2, 1) + u * Dskip[None, None, :]
        return y

    a = _A_ref(A_x, A_wqkv, A_wo)
    b = _B_ref(B_u, B_A_re, B_A_im, B_B_re, B_B_im, B_C_re, B_C_im, B_log_dt, B_Dskip)
    return jnp.concatenate([a, b], axis=-1)
```

```python
import math
import cmath
import jax
import jax.numpy as jnp
from jax import lax
import jax.experimental.pallas as pl
import jax.experimental.pallas.tpu as pltpu

f32 = jnp.float32
bf16 = jnp.bfloat16
NT = (((1,), (1,)), ((), ()))

S, D, H, DH, W = 2048, 512, 32, 16, 256
QB = 128
WIN = QB + W
HG = 8
NG = H // HG
NSTEP = (S // QB) * NG
L, NM = 2048, 128
KU, FU = 16, 4

def sincos(x):
    kf = jnp.floor(x * 0.6366197723675814 + 0.5)
    r = x - kf * 1.5703125
    r = r - kf * 4.837512969970703125e-4
    r = r - kf * 7.54978995489188216e-8
    q = kf.astype(jnp.int32) & 3
    r2 = r * r
    s = r + r * r2 * (-1.6666654611e-1 + r2 * (8.3321608736e-3 + r2 * (-1.9515295891e-4)))
    c = 1.0 - 0.5 * r2 + r2 * r2 * (4.166664568298827e-2 + r2 * (-1.388731625493765e-3 + r2 * 2.443315711809948e-5))
    swap = (q & 1) == 1
    sn = jnp.where(swap, c, s)
    cs = jnp.where(swap, s, c)
    sn = jnp.where(q >= 2, -sn, sn)
    cs = jnp.where((q == 1) | (q == 2), -cs, cs)
    return sn, cs

def cexp(zr, zi):
    e = jnp.exp(zr)
    s, c = sincos(zi)
    return e * c, e * s

def cmul(ar, ai, br, bi):
    return ar * br - ai * bi, ar * bi + ai * br

def cmulc(a, w):
    ar, ai = a
    if abs(w - 1) < 1e-12: return a
    if abs(w + 1) < 1e-12: return (-ar, -ai)
    if abs(w + 1j) < 1e-12: return (ai, -ar)
    if abs(w - 1j) < 1e-12: return (-ai, ar)
    wr, wi = float(w.real), float(w.imag)
    return (ar * wr - ai * wi, ar * wi + ai * wr)

def fft_list(x, sign):
    n = len(x)
    if n == 1: return x
    e = fft_list(x[0::2], sign); o = fft_list(x[1::2], sign)
    out = [None] * n
    for k in range(n // 2):
        t = cmulc(o[k], cmath.exp(sign * 2j * math.pi * k / n))
        out[k] = (e[k][0] + t[0], e[k][1] + t[1])
        out[k + n // 2] = (e[k][0] - t[0], e[k][1] - t[1])
    return out


def fused_kernel(x_ref, wqkv_ref, wo_ref, u_ref, are_ref, aim_ref, bre_ref, bim_ref, cre_ref, cim_ref, ldt_ref, dsk_ref,
                 o_ref,
                 q_s, k_s, vT_s, oT_s, mask_s, sA, sB, mA, mB,
                 par, R, uf, Wf, PU, PK, yf, tw):
    k_s[0:W, :] = jnp.zeros((W, D), bf16)
    vT_s[:, 0:W] = jnp.zeros((D, W), bf16)
    wvT = wqkv_ref[:, 2 * D:3 * D].T
    CH = 256
    def proj(c, carry):
        r0 = pl.multiple_of(c * CH, CH)
        xc = x_ref[pl.ds(r0, CH), :]
        qk = jnp.dot(xc, wqkv_ref[:, 0:2 * D], preferred_element_type=f32)
        q_s[pl.ds(r0, CH), :] = (qk[:, 0:D] * 0.25).astype(bf16)
        k_s[pl.ds(W + r0, CH), :] = qk[:, D:2 * D].astype(bf16)
        vT = lax.dot_general(wvT, xc, NT, preferred_element_type=f32)
        vT_s[:, pl.ds(W + r0, CH)] = vT.astype(bf16)
        return carry
    lax.fori_loop(0, S // CH, proj, 0)

    r = lax.broadcasted_iota(jnp.int32, (WIN, QB), 0)
    cq = lax.broadcasted_iota(jnp.int32, (WIN, QB), 1)
    for v in range(3):
        valid = (r > cq) & (r - W <= cq) & (r >= W - v * QB)
        mask_s[v] = jnp.where(valid, 0.0, -1e9).astype(f32)

    lane_head = lax.broadcasted_iota(jnp.int32, (QB, 128), 1) // DH
    ones_rows = jnp.ones((16, WIN), bf16)

    def qk_stage(t, s_buf, m_buf):
        qb = t // NG
        g = t % NG
        q0 = pl.multiple_of(qb * QB, QB)
        g0 = pl.multiple_of(g * 128, 128)
        qg = q_s[pl.ds(q0, QB), pl.ds(g0, 128)]
        kg = k_s[pl.ds(q0, WIN), pl.ds(g0, 128)]
        qm = jnp.concatenate([jnp.where(lane_head == hh, qg, jnp.zeros_like(qg)) for hh in range(HG)], axis=0)
        sT_all = lax.dot_general(kg, qm, NT, preferred_element_type=f32)
        bias = mask_s[jnp.minimum(qb, 2)]
        for hh in range(HG):
            sT = sT_all[:, hh * QB:(hh + 1) * QB] + bias
            m_buf[:, hh * QB:(hh + 1) * QB] = jnp.max(sT, axis=0, keepdims=True)
            s_buf[:, hh * QB:(hh + 1) * QB] = sT

    def sm_stage(t, s_buf, m_buf):
        qb = t // NG
        g = t % NG
        q0 = pl.multiple_of(qb * QB, QB)
        for hh in range(HG):
            sT = s_buf[:, hh * QB:(hh + 1) * QB]
            m = m_buf[:, hh * QB:(hh + 1) * QB]
            p = jnp.exp(sT - m).astype(bf16)
            h0 = pl.multiple_of((g * HG + hh) * DH, DH)
            vh = vT_s[pl.ds(h0, DH), pl.ds(q0, WIN)]
            lhs = jnp.concatenate([vh, ones_rows], axis=0)
            oT = jnp.dot(lhs, p, preferred_element_type=f32)
            res = oT[0:DH, :] / oT[DH:DH + 1, :]
            oT_s[pl.ds(h0, DH), pl.ds(q0, QB)] = res.astype(bf16)

    qk_stage(0, sA, mA)
    def body(i, carry):
        t0 = 2 * i
        qk_stage(t0 + 1, sB, mB)
        sm_stage(t0, sA, mA)
        qk_stage(jnp.minimum(t0 + 2, NSTEP - 1), sA, mA)
        sm_stage(t0 + 1, sB, mB)
        return carry
    lax.fori_loop(0, NSTEP // 2, body, 0)

    def outp(c, carry):
        r0 = pl.multiple_of(c * CH, CH)
        o = oT_s[:, pl.ds(r0, CH)].T
        o_ref[pl.ds(r0, CH), 0:D] = jnp.dot(o, wo_ref[...], preferred_element_type=f32).astype(o_ref.dtype)
        return carry
    lax.fori_loop(0, S // CH, outp, 0)

    dt = jnp.exp(ldt_ref[...].astype(f32)).astype(bf16).astype(f32)
    zr = are_ref[...].astype(f32) * dt
    zi = aim_ref[...].astype(f32) * dt
    dbr = bre_ref[...].astype(f32) * dt
    dbi = bim_ref[...].astype(f32) * dt
    cr, ci = cmul(cre_ref[...].astype(f32), cim_ref[...].astype(f32), dbr, dbi)
    par[0] = cr; par[1] = ci
    def csq(ar, ai):
        return ar * ar - ai * ai, 2.0 * ar * ai
    a1 = cexp(zr, zi); a2 = csq(*a1); a4 = csq(*a2); a8 = cexp(zr * 8, zi * 8)
    a32 = cexp(zr * 32, -zi * 32); a64 = csq(*a32); a128 = csq(*a64); a256 = cexp(zr * 256, -zi * 256)
    for idx, a in enumerate([a1, a2, a4, a8, a32, a64, a128, a256]):
        par[2 + 2 * idx] = a[0]; par[3 + 2 * idx] = a[1]

    sub = lax.broadcasted_iota(jnp.int32, (8, NM), 0)
    b0 = (sub & 1) == 1; b1 = (sub & 2) == 2; b2 = (sub & 4) == 4
    lane = lax.broadcasted_iota(jnp.int32, (40, 128), 1)
    def row(k, d):
        return par[k, pl.ds(d, 1), :]
    def pow8(d, k0):
        f0 = (jnp.where(b0, row(k0, d), 1.0), jnp.where(b0, row(k0 + 1, d), 0.0))
        f1 = (jnp.where(b1, row(k0 + 2, d), 1.0), jnp.where(b1, row(k0 + 3, d), 0.0))
        f2 = (jnp.where(b2, row(k0 + 4, d), 1.0), jnp.where(b2, row(k0 + 5, d), 0.0))
        t = cmul(*f0, *f1)
        return cmul(*t, *f2)
    def chan(d):
        lo = pow8(d, 2)
        T = cmul(row(0, d), row(1, d), *lo)
        Tr, Ti = [T[0]], [T[1]]
        a8r, a8i = row(8, d), row(9, d)
        for b in range(4):
            T = cmul(*T, a8r, a8i); Tr.append(T[0]); Ti.append(T[1])
        P = pow8(d, 10)
        Pr, Pi = [P[0]], [P[1]]
        a256r, a256i = row(16, d), row(17, d)
        for b in range(7):
            P = cmul(*P, a256r, a256i); Pr.append(P[0]); Pi.append(P[1])
        lhs = jnp.concatenate([jnp.concatenate(Tr, 0), jnp.concatenate(Ti, 0)], 1)
        rhs = jnp.concatenate([jnp.concatenate(Pr, 0), jnp.concatenate(Pi, 0)], 1)
        return lhs, rhs
    def kgen(c, carry):
        l0, r0 = chan(c)
        l1, r1 = chan(c + 256)
        lhs = jnp.concatenate([l0, l1], 0).astype(bf16)
        rhs = jnp.concatenate([r0, r1], 0).astype(bf16)
        out = lax.dot_general(lhs, rhs, NT, preferred_element_type=f32)
        R[pl.ds(c, 40, stride=256), :] = jnp.where(lane < 64, out[0:40], out[40:80])
        return carry
    lax.fori_loop(0, 256, kgen, 0, unroll=KU)

    rr = lax.broadcasted_iota(jnp.int32, (128, 128), 0)
    cc = lax.broadcasted_iota(jnp.int32, (128, 128), 1)
    same = (rr >= 64) == (cc >= 64)
    ii = rr & 63; kk = cc & 63
    n = (ii * (2 * kk + 1)) & 255
    sA, cA = sincos(n.astype(f32) * (2.0 * math.pi / 256))
    Ar = jnp.where(same, cA, 0.0); Ai = jnp.where(same, -sA, 0.0)
    jb = lax.broadcasted_iota(jnp.int32, (32, 128), 0)
    kb_ = lax.broadcasted_iota(jnp.int32, (32, 128), 1) & 63
    sB, cB = sincos((jb * (2 * kb_ + 1)).astype(f32) * (2.0 * math.pi / 8192))
    tw[0:32, :] = cB
    tw[32:64, :] = -sB
    def wgen(j, carry):
        Br = tw[pl.ds(j, 1), :]; Bi = tw[pl.ds(32 + j, 1), :]
        wr, wi = cmul(Ar, Ai, Br, Bi)
        Wf[pl.ds(pl.multiple_of(j * 128, 128), 128), :] = jnp.concatenate([wr, wi], 1).astype(bf16)
        return carry
    lax.fori_loop(0, 32, wgen, 0)

    for b in range(4):
        uf[pl.ds(b * L, L), :] = u_ref[:, b * 128:(b + 1) * 128].astype(f32)
    li = lax.broadcasted_iota(jnp.int32, (256, 128), 1) & 63
    def fwd(j, carry):
        blocks = []
        for beta in range(2):
            B = jnp.concatenate([uf[pl.ds(beta * L + j, 64, stride=32), :],
                                 uf[pl.ds((2 + beta) * L + j, 64, stride=32), :]], 0)
            blocks.append(B.T)
        Su = jnp.concatenate(blocks, 0).astype(bf16)
        def slab(s):
            t = j if s == 0 else ((j + (1 << (s - 1)) - 1 + ((j >> s) & 1)) >> s) << s
            return R[pl.ds(pl.multiple_of(t * 256, 256), 256), :]
        Sk = jnp.where(li < 8, slab(0), jnp.where(li < 16, slab(1), jnp.where(li < 32, slab(2), slab(3)))).astype(bf16)
        P = jnp.dot(jnp.concatenate([Su, Sk], 0), Wf[pl.ds(pl.multiple_of(j * 128, 128), 128), :], preferred_element_type=f32)
        PU[j] = P[0:256]
        PK[j] = P[256:512]
        return carry
    lax.fori_loop(0, 32, fwd, 0, unroll=FU)

    def ld(ref, slot, r0):
        return (ref[slot, pl.ds(r0, 8), 0:128], ref[slot, pl.ds(r0, 8), 128:256])
    def st(ref, slot, r0, v):
        ref[slot, pl.ds(r0, 8), 0:128] = v[0]
        ref[slot, pl.ds(r0, 8), 128:256] = v[1]
    def vpu(ch, carry):
        r0 = pl.multiple_of(ch * 8, 8)
        for ref in (PU, PK):
            for j0 in range(4):
                a = fft_list([ld(ref, 4 * j1 + j0, r0) for j1 in range(8)], -1)
                for k0 in range(8):
                    st(ref, 4 * k0 + j0, r0, cmulc(a[k0], cmath.exp(-2j * math.pi * j0 * k0 / 32)))
        for k0 in range(8):
            xu = fft_list([ld(PU, 4 * k0 + j0, r0) for j0 in range(4)], -1)
            xk = fft_list([ld(PK, 4 * k0 + j0, r0) for j0 in range(4)], -1)
            y = [cmul(*xu[k1], *xk[k1]) for k1 in range(4)]
            b = fft_list(y, +1)
            for j0 in range(4):
                st(PU, 4 * k0 + j0, r0, cmulc(b[j0], cmath.exp(2j * math.pi * j0 * k0 / 32)))
        for j0 in range(4):
            z = fft_list([ld(PU, 4 * k0 + j0, r0) for k0 in range(8)], +1)
            for j1 in range(8):
                st(PU, 4 * j1 + j0, r0, z[j1])
        return carry
    lax.fori_loop(0, 32, vpu, 0)

    def inv(j, carry):
        Z = PU[j].astype(bf16)
        O = lax.dot_general(Z, Wf[pl.ds(pl.multiple_of(j * 128, 128), 128), :], NT, preferred_element_type=f32) * (2.0 / 4096)
        for beta in range(2):
            T = O[beta * 128:(beta + 1) * 128, :].T
            j64 = pl.multiple_of(j * 64, 64)
            yf[pl.ds(beta * L + j64, 64), :] = T[0:64]
            yf[pl.ds((2 + beta) * L + j64, 64), :] = T[64:128]
        return carry
    lax.fori_loop(0, 32, inv, 0, unroll=FU)

    def fin(i, carry):
        r0 = pl.multiple_of(i * 32, 32)
        for b in range(4):
            yb = yf[pl.ds(b * L + i, 32, stride=64), :].astype(bf16)
            ub = u_ref[pl.ds(r0, 32), b * 128:(b + 1) * 128]
            o_ref[pl.ds(r0, 32), D + b * 128:D + (b + 1) * 128] = yb + ub * dsk_ref[:, b * 128:(b + 1) * 128]
        return carry
    lax.fori_loop(0, 64, fin, 0, unroll=4)


@jax.jit
def pallas_concat_heads__sliding_block__ssm_conv_s4__prompt_kernel(
    A_x: jax.Array,
    A_wqkv: jax.Array,
    A_wo: jax.Array,
    B_u: jax.Array,
    B_A_re: jax.Array,
    B_A_im: jax.Array,
    B_B_re: jax.Array,
    B_B_im: jax.Array,
    B_C_re: jax.Array,
    B_C_im: jax.Array,
    B_log_dt: jax.Array,
    B_Dskip: jax.Array,
):
    out = pl.pallas_call(
        fused_kernel,
        out_shape=jax.ShapeDtypeStruct((S, 2 * D), bf16),
        scratch_shapes=[
            pltpu.VMEM((S, D), bf16),
            pltpu.VMEM((S + W, D), bf16),
            pltpu.VMEM((D, S + W), bf16),
            pltpu.VMEM((D, S), bf16),
            pltpu.VMEM((3, WIN, QB), f32),
            pltpu.VMEM((WIN, HG * QB), f32),
            pltpu.VMEM((WIN, HG * QB), f32),
            pltpu.VMEM((1, HG * QB), f32),
            pltpu.VMEM((1, HG * QB), f32),
            pltpu.VMEM((18, D, NM), f32),
            pltpu.VMEM((40 * 256, 128), f32),
            pltpu.VMEM((4 * L, 128), f32),
            pltpu.VMEM((32 * 128, 256), bf16),
            pltpu.VMEM((32, 256, 256), f32),
            pltpu.VMEM((32, 256, 256), f32),
            pltpu.VMEM((4 * L, 128), f32),
            pltpu.VMEM((64, 128), f32),
        ],
        compiler_params=pltpu.CompilerParams(vmem_limit_bytes=100 * 1024 * 1024),
    )(A_x[0], A_wqkv, A_wo, B_u[0], B_A_re, B_A_im, B_B_re, B_B_im, B_C_re, B_C_im,
      B_log_dt.reshape(D, 1), B_Dskip.reshape(1, D))
    return out[None]
```

```python
import math
import cmath
import jax
import jax.numpy as jnp
from jax import lax
import jax.experimental.pallas as pl
import jax.experimental.pallas.tpu as pltpu

f32 = jnp.float32
bf16 = jnp.bfloat16
NT = (((1,), (1,)), ((), ()))

S, D, H, DH, W = 2048, 512, 32, 16, 256
QB = 64
WIN = QB + W
NQB = S // QB
NSTEP = (S // 128) * 4
CH = 256
L, NM = 2048, 128
KU, FU = 16, 4


def sincos(x):
    kf = jnp.floor(x * 0.6366197723675814 + 0.5)
    r = x - kf * 1.5703125
    r = r - kf * 4.837512969970703125e-4
    r = r - kf * 7.54978995489188216e-8
    q = kf.astype(jnp.int32) & 3
    r2 = r * r
    s = r + r * r2 * (-1.6666654611e-1 + r2 * (8.3321608736e-3 + r2 * (-1.9515295891e-4)))
    c = 1.0 - 0.5 * r2 + r2 * r2 * (4.166664568298827e-2 + r2 * (-1.388731625493765e-3 + r2 * 2.443315711809948e-5))
    swap = (q & 1) == 1
    sn = jnp.where(swap, c, s)
    cs = jnp.where(swap, s, c)
    sn = jnp.where(q >= 2, -sn, sn)
    cs = jnp.where((q == 1) | (q == 2), -cs, cs)
    return sn, cs


def cexp(zr, zi):
    e = jnp.exp(zr)
    s, c = sincos(zi)
    return e * c, e * s


def cmul(ar, ai, br, bi):
    return ar * br - ai * bi, ar * bi + ai * br


def csq(ar, ai):
    return ar * ar - ai * ai, 2.0 * ar * ai


def cmulc(a, w):
    ar, ai = a
    if abs(w - 1) < 1e-12:
        return a
    if abs(w + 1) < 1e-12:
        return (-ar, -ai)
    if abs(w + 1j) < 1e-12:
        return (ai, -ar)
    if abs(w - 1j) < 1e-12:
        return (-ai, ar)
    wr, wi = float(w.real), float(w.imag)
    return (ar * wr - ai * wi, ar * wi + ai * wr)


def fft_list(x, sign):
    n = len(x)
    if n == 1:
        return x
    e = fft_list(x[0::2], sign)
    o = fft_list(x[1::2], sign)
    out = [None] * n
    for k in range(n // 2):
        t = cmulc(o[k], cmath.exp(sign * 2j * math.pi * k / n))
        out[k] = (e[k][0] + t[0], e[k][1] + t[1])
        out[k + n // 2] = (e[k][0] - t[0], e[k][1] - t[1])
    return out


def fused_kernel(x_hbm, wqkv_hbm, wo_hbm, u_hbm, are_ref, aim_ref, bre_ref, bim_ref, cre_ref, cim_ref, ldt_ref, dsk_in,
                 out_hbm,
                 x_ref, wqkv_ref, wo_ref, u_ref, o_ref, isem, osem,
                 q_s, k_s, vT_s, oT_s, mask_s, sA, sB, mA, mB,
                 par, R, uf, Wf, PU, PK, yf, tw, SU):
    cp_u = pltpu.make_async_copy(u_hbm, u_ref, isem.at[0])
    cp_x = pltpu.make_async_copy(x_hbm, x_ref, isem.at[1])
    cp_w = pltpu.make_async_copy(wqkv_hbm, wqkv_ref, isem.at[2])
    cp_o = pltpu.make_async_copy(wo_hbm, wo_ref, isem.at[3])
    cp_u.start(); cp_x.start(); cp_w.start(); cp_o.start()
    dsk_row = dsk_in[...].reshape(1, D)
    dt = jnp.exp(ldt_ref[...].astype(f32)).astype(bf16).astype(f32).reshape(1, D)
    dt = jnp.broadcast_to(dt, (NM, D)).T
    zr = are_ref[...].astype(f32) * dt
    zi = aim_ref[...].astype(f32) * dt
    cr, ci = cmul(cre_ref[...].astype(f32), cim_ref[...].astype(f32),
                  bre_ref[...].astype(f32) * dt, bim_ref[...].astype(f32) * dt)
    par[0] = cr
    par[1] = ci
    a1 = cexp(zr, zi)
    a2 = csq(*a1)
    par[2] = a1[0]; par[3] = a1[1]
    par[4] = a2[0]; par[5] = a2[1]
    a4 = csq(*a2)
    par[6] = a4[0]; par[7] = a4[1]
    a8 = cexp(zr * 8, zi * 8)
    par[8] = a8[0]; par[9] = a8[1]
    a32 = cexp(zr * 32, -zi * 32)
    par[10] = a32[0]; par[11] = a32[1]
    a64 = csq(*a32)
    par[12] = a64[0]; par[13] = a64[1]
    a128 = csq(*a64)
    par[14] = a128[0]; par[15] = a128[1]
    a256 = cexp(zr * 256, -zi * 256)
    par[16] = a256[0]; par[17] = a256[1]

    rr = lax.broadcasted_iota(jnp.int32, (128, 128), 0)
    cc = lax.broadcasted_iota(jnp.int32, (128, 128), 1)
    same = (rr >= 64) == (cc >= 64)
    nA = ((rr & 63) * (2 * (cc & 63) + 1)) & 255
    sA_, cA_ = sincos(nA.astype(f32) * (2.0 * math.pi / 256))
    Ar = jnp.where(same, cA_, 0.0)
    Ai = jnp.where(same, -sA_, 0.0)
    jb = lax.broadcasted_iota(jnp.int32, (32, 128), 0)
    kb = lax.broadcasted_iota(jnp.int32, (32, 128), 1) & 63
    sB_, cB_ = sincos((jb * (2 * kb + 1)).astype(f32) * (2.0 * math.pi / 8192))
    tw[0:32, :] = cB_
    tw[32:64, :] = -sB_

    def wgen(j, carry):
        wr, wi = cmul(Ar, Ai, tw[pl.ds(j, 1), :], tw[pl.ds(32 + j, 1), :])
        Wf[pl.ds(pl.multiple_of(j * 128, 128), 128), :] = jnp.concatenate([wr, wi], 1).astype(bf16)
        return carry
    lax.fori_loop(0, 32, wgen, 0)

    cp_u.wait()
    for b in range(4):
        uf[pl.ds(b * L, L), :] = u_ref[:, b * 128:(b + 1) * 128].astype(f32)

    sub = lax.broadcasted_iota(jnp.int32, (8, NM), 0)
    b0 = (sub & 1) == 1
    b1 = (sub & 2) == 2
    b2 = (sub & 4) == 4
    lane40 = lax.broadcasted_iota(jnp.int32, (40, 128), 1)

    def row(k, d):
        return par[k, pl.ds(d, 1), :]

    def pow8(d, k0):
        f0 = (jnp.where(b0, row(k0, d), 1.0), jnp.where(b0, row(k0 + 1, d), 0.0))
        f1 = (jnp.where(b1, row(k0 + 2, d), 1.0), jnp.where(b1, row(k0 + 3, d), 0.0))
        f2 = (jnp.where(b2, row(k0 + 4, d), 1.0), jnp.where(b2, row(k0 + 5, d), 0.0))
        return cmul(*cmul(*f0, *f1), *f2)

    def chan(d):
        T = cmul(row(0, d), row(1, d), *pow8(d, 2))
        Tr, Ti = [T[0]], [T[1]]
        for _ in range(4):
            T = cmul(*T, row(8, d), row(9, d))
            Tr.append(T[0]); Ti.append(T[1])
        P = pow8(d, 10)
        Pr, Pi = [P[0]], [P[1]]
        for _ in range(7):
            P = cmul(*P, row(16, d), row(17, d))
            Pr.append(P[0]); Pi.append(P[1])
        lhs = jnp.concatenate([jnp.concatenate(Tr, 0), jnp.concatenate(Ti, 0)], 1)
        rhs = jnp.concatenate([jnp.concatenate(Pr, 0), jnp.concatenate(Pi, 0)], 1)
        return lhs, rhs

    def kgen_pair(c):
        l0, r0 = chan(c)
        l1, r1 = chan(c + 256)
        lhs = jnp.concatenate([l0, l1], 0).astype(bf16)
        rhs = jnp.concatenate([r0, r1], 0).astype(bf16)
        out = lax.dot_general(lhs, rhs, NT, preferred_element_type=f32)
        R[pl.ds(c, 40, stride=256), :] = jnp.where(lane40 < 64, out[0:40], out[40:80])

    def ugather(j):
        for beta in range(2):
            blk = jnp.concatenate([uf[pl.ds(beta * L + j, 64, stride=32), :],
                                   uf[pl.ds((2 + beta) * L + j, 64, stride=32), :]], 0)
            SU[pl.ds(pl.multiple_of(j * 256 + beta * 128, 128), 128), :] = blk.T.astype(bf16)

    def kgen(it, carry):
        for p in range(KU):
            kgen_pair(it * KU + p)
        ugather(2 * it)
        ugather(2 * it + 1)
        return carry
    lax.fori_loop(0, 256 // KU, kgen, 0)

    li = lax.broadcasted_iota(jnp.int32, (256, 128), 1) & 63

    def fwd(j, carry):
        def slab(s):
            t = j if s == 0 else ((j + (1 << (s - 1)) - 1 + ((j >> s) & 1)) >> s) << s
            return R[pl.ds(pl.multiple_of(t * 256, 256), 256), :]
        Sk = jnp.where(li < 8, slab(0), jnp.where(li < 16, slab(1), jnp.where(li < 32, slab(2), slab(3)))).astype(bf16)
        Su = SU[pl.ds(pl.multiple_of(j * 256, 256), 256), :]
        P = jnp.dot(jnp.concatenate([Su, Sk], 0), Wf[pl.ds(pl.multiple_of(j * 128, 128), 128), :],
                    preferred_element_type=f32)
        PU[j] = P[0:256]
        PK[j] = P[256:512]
        return carry
    lax.fori_loop(0, 32, fwd, 0, unroll=FU)

    def ld(ref, slot, r0):
        return (ref[slot, pl.ds(r0, 8), 0:128], ref[slot, pl.ds(r0, 8), 128:256])

    def st(ref, slot, r0, v):
        ref[slot, pl.ds(r0, 8), 0:128] = v[0]
        ref[slot, pl.ds(r0, 8), 128:256] = v[1]

    def vpu(ch):
        r0 = pl.multiple_of(ch * 8, 8)
        for ref in (PU, PK):
            for j0 in range(4):
                a = fft_list([ld(ref, 4 * j1 + j0, r0) for j1 in range(8)], -1)
                for k0 in range(8):
                    st(ref, 4 * k0 + j0, r0, cmulc(a[k0], cmath.exp(-2j * math.pi * j0 * k0 / 32)))
        for k0 in range(8):
            xu = fft_list([ld(PU, 4 * k0 + j0, r0) for j0 in range(4)], -1)
            xk = fft_list([ld(PK, 4 * k0 + j0, r0) for j0 in range(4)], -1)
            y = [cmul(*xu[k1], *xk[k1]) for k1 in range(4)]
            bb = fft_list(y, +1)
            for j0 in range(4):
                st(PU, 4 * k0 + j0, r0, cmulc(bb[j0], cmath.exp(2j * math.pi * j0 * k0 / 32)))
        for j0 in range(4):
            z = fft_list([ld(PU, 4 * k0 + j0, r0) for k0 in range(8)], +1)
            for j1 in range(8):
                st(PU, 4 * j1 + j0, r0, z[j1])

    def inv(j):
        Z = PU[j].astype(bf16)
        O = lax.dot_general(Z, Wf[pl.ds(pl.multiple_of(j * 128, 128), 128), :], NT,
                            preferred_element_type=f32) * (2.0 / 4096)
        j64 = pl.multiple_of(j * 64, 64)
        for beta in range(2):
            T = O[beta * 128:(beta + 1) * 128, :].T
            yf[pl.ds(beta * L + j64, 64), :] = T[0:64]
            yf[pl.ds((2 + beta) * L + j64, 64), :] = T[64:128]

    def fin(i):
        r0 = pl.multiple_of(i * 32, 32)
        for b in range(4):
            yb = yf[pl.ds(b * L + i, 32, stride=64), :].astype(bf16)
            ub = u_ref[pl.ds(r0, 32), b * 128:(b + 1) * 128]
            o_ref[pl.ds(r0, 32), D + b * 128:D + (b + 1) * 128] = yb + ub * dsk_row[:, b * 128:(b + 1) * 128]

    cp_x.wait(); cp_w.wait()
    k_s[0:W, :] = jnp.zeros((W, D), bf16)
    vT_s[:, 0:W] = jnp.zeros((D, W), bf16)
    wvT = wqkv_ref[:, 2 * D:3 * D].T

    def proj_piece(c, n):
        r0 = pl.multiple_of(c * CH, CH)
        xc = x_ref[pl.ds(r0, CH), :]
        if n < 4:
            y = jnp.dot(xc, wqkv_ref[:, n * 256:(n + 1) * 256], preferred_element_type=f32)
            if n < 2:
                q_s[pl.ds(r0, CH), n * 256:(n + 1) * 256] = (y * 0.25).astype(bf16)
            else:
                k_s[pl.ds(W + r0, CH), (n - 2) * 256:(n - 1) * 256] = y.astype(bf16)
        else:
            m0 = (n - 4) * 256
            vT = lax.dot_general(wvT[m0:m0 + 256], xc, NT, preferred_element_type=f32)
            vT_s[m0:m0 + 256, pl.ds(W + r0, CH)] = vT.astype(bf16)

    def proj_vpu(c, carry):
        for qq in range(6):
            proj_piece(c, qq)
            if qq < 4:
                vpu(4 * c + qq)
        return carry
    lax.fori_loop(0, S // CH, proj_vpu, 0)

    rI = lax.broadcasted_iota(jnp.int32, (WIN, 128), 0)
    cq = lax.broadcasted_iota(jnp.int32, (WIN, 128), 1) & (QB - 1)
    for v in range(5):
        valid = (rI > cq) & (rI - W <= cq) & (rI >= W - v * QB)
        mask_s[v] = jnp.where(valid, 0.0, -1e9).astype(f32)

    lane_head = lax.broadcasted_iota(jnp.int32, (QB // 2, 128), 1) // DH
    lane16 = lax.broadcasted_iota(jnp.int32, (DH, 128), 1)

    def qk_stage(t, s_buf, m_buf):
        qp = t // 4
        g = t % 4
        q0 = pl.multiple_of(qp * 128, 128)
        g0 = pl.multiple_of(g * 128, 128)
        kg = k_s[pl.ds(q0, WIN + QB), pl.ds(g0, 128)]
        for e in range(2):
            qg = pltpu.bitcast(q_s[pl.ds(q0 + e * QB, QB), pl.ds(g0, 128)], jnp.uint32)
            qm = jnp.concatenate([pltpu.bitcast(jnp.where(lane_head == hh, qg, jnp.uint32(0)), bf16) for hh in range(8)], axis=0)
            sT_all = lax.dot_general(kg[e * QB:e * QB + WIN], qm, NT, preferred_element_type=f32)
            bias = mask_s[jnp.minimum(2 * qp + e, 4)]
            for tt in range(4):
                c0 = (e * 4 + tt) * 128
                sT = sT_all[:, tt * 128:(tt + 1) * 128] + bias
                m_buf[:, c0:c0 + 128] = jnp.max(sT, axis=0, keepdims=True)
                s_buf[:, c0:c0 + 128] = sT

    def sm_stage(t, s_buf, m_buf):
        qp = t // 4
        g = t % 4
        q0 = pl.multiple_of(qp * 128, 128)
        for tt in range(4):
            h0 = pl.multiple_of((g * 8 + 2 * tt) * DH, 2 * DH)
            vh = vT_s[pl.ds(h0, 2 * DH), pl.ds(q0, WIN + QB)]
            oTs = []
            for e in range(2):
                c0 = (e * 4 + tt) * 128
                p = jnp.exp(s_buf[:, c0:c0 + 128] - m_buf[:, c0:c0 + 128])
                l = jnp.sum(p, axis=0, keepdims=True)
                oTs.append(jnp.dot(vh[:, e * QB:e * QB + WIN], p.astype(bf16), preferred_element_type=f32) / l)
            low = lane16 < QB
            oT_s[pl.ds(h0, DH), pl.ds(q0, 128)] = jnp.where(low, oTs[0][0:DH], pltpu.roll(oTs[1][0:DH], QB, 1)).astype(bf16)
            oT_s[pl.ds(h0 + DH, DH), pl.ds(q0, 128)] = jnp.where(low, pltpu.roll(oTs[0][DH:2 * DH], QB, 1), oTs[1][DH:2 * DH]).astype(bf16)

    def attn_pair(i):
        t0 = 2 * i
        qk_stage(t0 + 1, sB, mB)
        sm_stage(t0, sA, mA)
        qk_stage(jnp.minimum(t0 + 2, NSTEP - 1), sA, mA)
        sm_stage(t0 + 1, sB, mB)

    qk_stage(0, sA, mA)

    def loop1(i, carry):
        attn_pair(i)
        inv(2 * i)
        inv(2 * i + 1)
        return carry
    lax.fori_loop(0, 16, loop1, 0)

    def loop2(i, carry):
        attn_pair(i)
        for ff in range(4):
            fin(4 * (i - 16) + ff)
        return carry
    lax.fori_loop(16, 32, loop2, 0)

    cp_ob = pltpu.make_async_copy(o_ref.at[:, D:2 * D], out_hbm.at[:, D:2 * D], osem.at[S // CH])
    cp_ob.start()
    cp_o.wait()

    def outp(c, carry):
        r0 = pl.multiple_of(c * CH, CH)
        o = oT_s[:, pl.ds(r0, CH)].T
        o_ref[pl.ds(r0, CH), 0:D] = jnp.dot(o, wo_ref[...], preferred_element_type=f32).astype(o_ref.dtype)
        pltpu.make_async_copy(o_ref.at[pl.ds(r0, CH), 0:D], out_hbm.at[pl.ds(r0, CH), 0:D], osem.at[c]).start()
        return carry
    lax.fori_loop(0, S // CH, outp, 0)
    cp_ob.wait()
    for c in range(S // CH):
        pltpu.make_async_copy(o_ref.at[pl.ds(c * CH, CH), 0:D], out_hbm.at[pl.ds(c * CH, CH), 0:D], osem.at[c]).wait()


@jax.jit
def pallas_concat_heads__sliding_block__ssm_conv_s4__prompt_kernel(
    A_x: jax.Array,
    A_wqkv: jax.Array,
    A_wo: jax.Array,
    B_u: jax.Array,
    B_A_re: jax.Array,
    B_A_im: jax.Array,
    B_B_re: jax.Array,
    B_B_im: jax.Array,
    B_C_re: jax.Array,
    B_C_im: jax.Array,
    B_log_dt: jax.Array,
    B_Dskip: jax.Array,
):
    out = pl.pallas_call(
        fused_kernel,
        out_shape=jax.ShapeDtypeStruct((S, 2 * D), bf16),
        in_specs=[pl.BlockSpec(memory_space=pl.ANY)] * 4 + [pl.BlockSpec(memory_space=pltpu.VMEM)] * 8,
        out_specs=pl.BlockSpec(memory_space=pl.ANY),
        scratch_shapes=[
            pltpu.VMEM((S, D), bf16),
            pltpu.VMEM((D, 3 * D), bf16),
            pltpu.VMEM((D, D), bf16),
            pltpu.VMEM((L, D), bf16),
            pltpu.VMEM((S, 2 * D), bf16),
            pltpu.SemaphoreType.DMA((4,)),
            pltpu.SemaphoreType.DMA((S // CH + 1,)),
            pltpu.VMEM((S, D), bf16),
            pltpu.VMEM((S + W, D), bf16),
            pltpu.VMEM((D, S + W), bf16),
            pltpu.VMEM((D, S), bf16),
            pltpu.VMEM((5, WIN, 128), f32),
            pltpu.VMEM((WIN, 16 * QB), f32),
            pltpu.VMEM((WIN, 16 * QB), f32),
            pltpu.VMEM((1, 16 * QB), f32),
            pltpu.VMEM((1, 16 * QB), f32),
            pltpu.VMEM((18, D, NM), f32),
            pltpu.VMEM((40 * 256, 128), f32),
            pltpu.VMEM((4 * L, 128), f32),
            pltpu.VMEM((32 * 128, 256), bf16),
            pltpu.VMEM((32, 256, 256), f32),
            pltpu.VMEM((32, 256, 256), f32),
            pltpu.VMEM((4 * L, 128), f32),
            pltpu.VMEM((64, 128), f32),
            pltpu.VMEM((32 * 256, 128), bf16),
        ],
        compiler_params=pltpu.CompilerParams(vmem_limit_bytes=100 * 1024 * 1024),
    )(A_x[0], A_wqkv, A_wo, B_u[0], B_A_re, B_A_im, B_B_re, B_B_im, B_C_re, B_C_im,
      B_log_dt, B_Dskip)
    return out[None]
```

```python
import math
import cmath
import jax
import jax.numpy as jnp
from jax import lax
import jax.experimental.pallas as pl
import jax.experimental.pallas.tpu as pltpu

f32 = jnp.float32
bf16 = jnp.bfloat16
NT = (((1,), (1,)), ((), ()))

S, D, H, DH, W = 2048, 512, 32, 16, 256
QB = 64
WIN = QB + W
NSTEP = (S // 128) * 4
CH = 256
QSCALE = 0.25 * 1.4426950408889634
L, NM = 2048, 128


def interleave(*streams):
    active = [[g, w] for g, w in streams]
    while active:
        for item in list(active):
            g, w = item
            for _ in range(w):
                try:
                    next(g)
                except StopIteration:
                    active.remove(item)
                    break


def drain(g):
    for _ in g:
        pass


def chain(*gens):
    for g in gens:
        yield from g


def sincos(x):
    kf = jnp.floor(x * 0.6366197723675814 + 0.5)
    r = x - kf * 1.5703125
    r = r - kf * 4.837512969970703125e-4
    r = r - kf * 7.54978995489188216e-8
    q = kf.astype(jnp.int32) & 3
    r2 = r * r
    s = r + r * r2 * (-1.6666654611e-1 + r2 * (8.3321608736e-3 + r2 * (-1.9515295891e-4)))
    c = 1.0 - 0.5 * r2 + r2 * r2 * (4.166664568298827e-2 + r2 * (-1.388731625493765e-3 + r2 * 2.443315711809948e-5))
    swap = (q & 1) == 1
    sn = jnp.where(swap, c, s)
    cs = jnp.where(swap, s, c)
    sn = jnp.where(q >= 2, -sn, sn)
    cs = jnp.where((q == 1) | (q == 2), -cs, cs)
    return sn, cs


def cexp(zr, zi):
    e = jnp.exp(zr)
    s, c = sincos(zi)
    return e * c, e * s


def cmul(ar, ai, br, bi):
    return ar * br - ai * bi, ar * bi + ai * br


def csq(ar, ai):
    return ar * ar - ai * ai, 2.0 * ar * ai


def cmulc(a, w):
    ar, ai = a
    if abs(w - 1) < 1e-12:
        return a
    if abs(w + 1) < 1e-12:
        return (-ar, -ai)
    if abs(w + 1j) < 1e-12:
        return (ai, -ar)
    if abs(w - 1j) < 1e-12:
        return (-ai, ar)
    wr, wi = float(w.real), float(w.imag)
    return (ar * wr - ai * wi, ar * wi + ai * wr)


def fft_g(x, sign):
    n = len(x)
    bits = n.bit_length() - 1
    a = [x[int(format(i, '0%db' % bits)[::-1], 2)] for i in range(n)]
    size = 2
    while size <= n:
        half = size // 2
        for start in range(0, n, size):
            for k in range(half):
                t = cmulc(a[start + k + half], cmath.exp(sign * 2j * math.pi * k / size))
                u = a[start + k]
                a[start + k] = (u[0] + t[0], u[1] + t[1])
                a[start + k + half] = (u[0] - t[0], u[1] - t[1])
        yield
        size *= 2
    return a


def fused_kernel(x_hbm, wqkv_hbm, wo_hbm, u_hbm, are_ref, aim_ref, bre_ref, bim_ref, cre_ref, cim_ref, ldt_ref, dsk_in,
                 out_hbm,
                 x_ref, wqkv_ref, wo_ref, u_ref, o_ref, isem, osem,
                 q_s, k_s, vT_s, oT_s, mask_s, sA, sB, mA, mB, wvT_s,
                 par, R, uf, Wf, PU, PK, yf, tw, SU):
    cp_x = pltpu.make_async_copy(x_hbm, x_ref, isem.at[1])
    cp_w = pltpu.make_async_copy(wqkv_hbm, wqkv_ref, isem.at[2])
    cp_u = pltpu.make_async_copy(u_hbm, u_ref, isem.at[0])
    cp_o = pltpu.make_async_copy(wo_hbm, wo_ref, isem.at[3])
    cp_w.start(); cp_x.start(); cp_u.start(); cp_o.start()
    dsk_row = dsk_in[...].reshape(1, D)

    dt = jnp.exp(ldt_ref[...].astype(f32)).astype(bf16).astype(f32).reshape(1, D)
    dt = jnp.broadcast_to(dt, (NM, D)).T
    zr = are_ref[...].astype(f32) * dt
    zi = aim_ref[...].astype(f32) * dt
    cr, ci = cmul(cre_ref[...].astype(f32), cim_ref[...].astype(f32),
                  bre_ref[...].astype(f32) * dt, bim_ref[...].astype(f32) * dt)
    par[0] = cr
    par[1] = ci
    a1 = cexp(zr, zi)
    a2 = csq(*a1)
    par[2] = a1[0]; par[3] = a1[1]
    par[4] = a2[0]; par[5] = a2[1]
    a4 = csq(*a2)
    par[6] = a4[0]; par[7] = a4[1]
    a8 = cexp(zr * 8, zi * 8)
    par[8] = a8[0]; par[9] = a8[1]
    a32 = cexp(zr * 32, -zi * 32)
    par[10] = a32[0]; par[11] = a32[1]
    a64 = csq(*a32)
    par[12] = a64[0]; par[13] = a64[1]
    a128 = csq(*a64)
    par[14] = a128[0]; par[15] = a128[1]
    a256 = cexp(zr * 256, -zi * 256)
    par[16] = a256[0]; par[17] = a256[1]

    rr = lax.broadcasted_iota(jnp.int32, (128, 128), 0)
    cc = lax.broadcasted_iota(jnp.int32, (128, 128), 1)
    same = (rr >= 64) == (cc >= 64)
    nA = ((rr & 63) * (2 * (cc & 63) + 1)) & 255
    sA_, cA_ = sincos(nA.astype(f32) * (2.0 * math.pi / 256))
    Ar = jnp.where(same, cA_, 0.0)
    Ai = jnp.where(same, -sA_, 0.0)
    jb = lax.broadcasted_iota(jnp.int32, (32, 128), 0)
    kb = lax.broadcasted_iota(jnp.int32, (32, 128), 1) & 63
    sB_, cB_ = sincos((jb * (2 * kb + 1)).astype(f32) * (2.0 * math.pi / 8192))
    tw[0:32, :] = cB_
    tw[32:64, :] = -sB_

    def wgen(j, carry):
        wr, wi = cmul(Ar, Ai, tw[pl.ds(j, 1), :], tw[pl.ds(32 + j, 1), :])
        Wf[pl.ds(pl.multiple_of(j * 128, 128), 128), :] = jnp.concatenate([wr, wi], 1).astype(bf16)
        return carry
    lax.fori_loop(0, 32, wgen, 0)

    rI = lax.broadcasted_iota(jnp.int32, (WIN, 128), 0)
    cq = lax.broadcasted_iota(jnp.int32, (WIN, 128), 1) & (QB - 1)
    for v in range(5):
        valid = (rI > cq) & (rI - W <= cq) & (rI >= W - v * QB)
        mask_s[v] = jnp.where(valid, 0.0, -1e9).astype(f32)
    for b in range(4):
        k_s[b, 0:W, :] = jnp.zeros((W, 128), bf16)
    vT_s[:, 0:W] = jnp.zeros((D, W), bf16)
    cp_w.wait()
    wvT_s[...] = wqkv_ref[:, 2 * D:3 * D].T
    cp_u.wait()
    for b in range(4):
        uf[pl.ds(b * L, L), :] = u_ref[:, b * 128:(b + 1) * 128].astype(f32)
    cp_x.wait()

    sub = lax.broadcasted_iota(jnp.int32, (8, NM), 0)
    b0 = (sub & 1) == 1
    b1 = (sub & 2) == 2
    b2 = (sub & 4) == 4
    lane40 = lax.broadcasted_iota(jnp.int32, (40, 128), 1)

    def row(k, d):
        return par[k, pl.ds(d, 1), :]

    def pow8(d, k0):
        f0 = (jnp.where(b0, row(k0, d), 1.0), jnp.where(b0, row(k0 + 1, d), 0.0))
        f1 = (jnp.where(b1, row(k0 + 2, d), 1.0), jnp.where(b1, row(k0 + 3, d), 0.0))
        f2 = (jnp.where(b2, row(k0 + 4, d), 1.0), jnp.where(b2, row(k0 + 5, d), 0.0))
        return cmul(*cmul(*f0, *f1), *f2)

    def chan_g(d):
        T = cmul(row(0, d), row(1, d), *pow8(d, 2))
        Tr, Ti = [T[0]], [T[1]]
        yield
        for _ in range(4):
            T = cmul(*T, row(8, d), row(9, d))
            Tr.append(T[0]); Ti.append(T[1])
        yield
        P = pow8(d, 10)
        Pr, Pi = [P[0]], [P[1]]
        yield
        for it in range(7):
            P = cmul(*P, row(16, d), row(17, d))
            Pr.append(P[0]); Pi.append(P[1])
            if it == 3:
                yield
        yield
        lhs = jnp.concatenate([jnp.concatenate(Tr, 0), jnp.concatenate(Ti, 0)], 1)
        rhs = jnp.concatenate([jnp.concatenate(Pr, 0), jnp.concatenate(Pi, 0)], 1)
        return lhs, rhs

    def kgen_pair_g(c):
        l0, r0 = yield from chan_g(c)
        l1, r1 = yield from chan_g(c + 256)
        lhs = jnp.concatenate([l0, l1], 0).astype(bf16)
        rhs = jnp.concatenate([r0, r1], 0).astype(bf16)
        out = lax.dot_general(lhs, rhs, NT, preferred_element_type=f32)
        R[pl.ds(c, 40, stride=256), :] = jnp.where(lane40 < 64, out[0:40], out[40:80])
        yield

    def ugather_g(j):
        for beta in range(2):
            blk = jnp.concatenate([uf[pl.ds(beta * L + j, 64, stride=32), :],
                                   uf[pl.ds((2 + beta) * L + j, 64, stride=32), :]], 0)
            yield
            SU[pl.ds(pl.multiple_of(j * 256 + beta * 128, 128), 128), :] = blk.T.astype(bf16)
            yield

    def proj_g(c):
        r0 = pl.multiple_of(c * CH, CH)
        for mh in range(CH // 128):
            xr = pl.ds(pl.multiple_of(r0 + mh * 128, 128), 128)
            kr = pl.ds(pl.multiple_of(W + r0 + mh * 128, 128), 128)
            for n in range(8):
                y = jnp.dot(x_ref[xr, :], wqkv_ref[:, n * 128:(n + 1) * 128], preferred_element_type=f32)
                if n < 4:
                    q_s[n, xr, :] = (y * QSCALE).astype(bf16)
                else:
                    k_s[n - 4, kr, :] = y.astype(bf16)
                yield
            for m in range(4):
                vT = lax.dot_general(wvT_s[m * 128:(m + 1) * 128, :], x_ref[xr, :], NT, preferred_element_type=f32)
                vT_s[m * 128:(m + 1) * 128, kr] = vT.astype(bf16)
                yield

    NPI = 256 // (S // CH)

    def kgen_proj(it, carry):
        kg = chain(*[chain(kgen_pair_g(it * NPI + p), *( [ugather_g(it * 4 + p // 8)] if p % 8 == 7 else [])) for p in range(NPI)])
        interleave((proj_g(it), 1), (kg, KW))
        return carry
    lax.fori_loop(0, S // CH, kgen_proj, 0)

    li = lax.broadcasted_iota(jnp.int32, (256, 128), 1) & 63

    def fwd(j, carry):
        def slab(s):
            t = j if s == 0 else ((j + (1 << (s - 1)) - 1 + ((j >> s) & 1)) >> s) << s
            return R[pl.ds(pl.multiple_of(t * 256, 256), 256), :]
        Sk = jnp.where(li < 8, slab(0), jnp.where(li < 16, slab(1), jnp.where(li < 32, slab(2), slab(3)))).astype(bf16)
        Su = SU[pl.ds(pl.multiple_of(j * 256, 256), 256), :]
        P = jnp.dot(jnp.concatenate([Su, Sk], 0), Wf[pl.ds(pl.multiple_of(j * 128, 128), 128), :],
                    preferred_element_type=f32)
        PU[j] = P[0:256]
        PK[j] = P[256:512]
        return carry
    lax.fori_loop(0, 32, fwd, 0, unroll=4)

    def ld(ref, slot, r0):
        return (ref[slot, pl.ds(r0, 8), 0:128], ref[slot, pl.ds(r0, 8), 128:256])

    def st(ref, slot, r0, v):
        ref[slot, pl.ds(r0, 8), 0:128] = v[0]
        ref[slot, pl.ds(r0, 8), 128:256] = v[1]

    def vpu_g(ch):
        r0 = pl.multiple_of(ch * 8, 8)
        for ref in (PU, PK):
            for j0 in range(4):
                a = yield from fft_g([ld(ref, 4 * j1 + j0, r0) for j1 in range(8)], -1)
                for k0 in range(8):
                    st(ref, 4 * k0 + j0, r0, cmulc(a[k0], cmath.exp(-2j * math.pi * j0 * k0 / 32)))
                yield
        for k0 in range(8):
            xu = yield from fft_g([ld(PU, 4 * k0 + j0, r0) for j0 in range(4)], -1)
            xk = yield from fft_g([ld(PK, 4 * k0 + j0, r0) for j0 in range(4)], -1)
            y = [cmul(*xu[k1], *xk[k1]) for k1 in range(4)]
            bb = yield from fft_g(y, +1)
            for j0 in range(4):
                st(PU, 4 * k0 + j0, r0, cmulc(bb[j0], cmath.exp(2j * math.pi * j0 * k0 / 32)))
            yield
        for j0 in range(4):
            z = yield from fft_g([ld(PU, 4 * k0 + j0, r0) for k0 in range(8)], +1)
            for j1 in range(8):
                st(PU, 4 * j1 + j0, r0, z[j1])
            yield

    def inv_g(j):
        Z = PU[j].astype(bf16)
        O = lax.dot_general(Z, Wf[pl.ds(pl.multiple_of(j * 128, 128), 128), :], NT,
                            preferred_element_type=f32) * (2.0 / 4096)
        yield
        j64 = pl.multiple_of(j * 64, 64)
        for beta in range(2):
            T = O[beta * 128:(beta + 1) * 128, :].T
            yf[pl.ds(beta * L + j64, 64), :] = T[0:64]
            yf[pl.ds((2 + beta) * L + j64, 64), :] = T[64:128]
            yield

    def fin_g(i):
        r0 = pl.multiple_of(i * 32, 32)
        for b in range(4):
            yb = yf[pl.ds(b * L + i, 32, stride=64), :].astype(bf16)
            ub = u_ref[pl.ds(r0, 32), b * 128:(b + 1) * 128]
            o_ref[pl.ds(r0, 32), D + b * 128:D + (b + 1) * 128] = yb + ub * dsk_row[:, b * 128:(b + 1) * 128]
            yield

    lane_head = lax.broadcasted_iota(jnp.int32, (QB // 2, 128), 1) // DH
    lane16 = lax.broadcasted_iota(jnp.int32, (DH, 128), 1)

    def qk_g(t, s_buf, m_buf, full_mask):
        qp = t // 4
        g = t % 4
        q0 = pl.multiple_of(qp * 128, 128)
        kg = k_s[g, pl.ds(q0, WIN + QB), :]
        for e in range(2):
            qg = pltpu.bitcast(q_s[g, pl.ds(q0 + e * QB, QB), :], jnp.uint32)
            qm = jnp.concatenate([pltpu.bitcast(jnp.where(lane_head == hh, qg, jnp.uint32(0)), bf16) for hh in range(8)], axis=0)
            sT_all = lax.dot_general(kg[e * QB:e * QB + WIN], qm, NT, preferred_element_type=f32)
            if full_mask:
                bias = mask_s[jnp.minimum(2 * qp + e, 4)]
            yield
            for tt in range(4):
                c0 = (e * 4 + tt) * 128
                if full_mask:
                    sT = sT_all[:, tt * 128:(tt + 1) * 128] + bias
                else:
                    sT = jnp.concatenate([sT_all[0:QB, tt * 128:(tt + 1) * 128] + mask_s[4, 0:QB, :],
                                          sT_all[QB:W, tt * 128:(tt + 1) * 128],
                                          sT_all[W:WIN, tt * 128:(tt + 1) * 128] + mask_s[4, W:WIN, :]], axis=0)
                m_buf[:, c0:c0 + 128] = jnp.max(sT, axis=0, keepdims=True)
                s_buf[:, c0:c0 + 128] = sT
                yield

    def sm_g(t, s_buf, m_buf):
        qp = t // 4
        g = t % 4
        q0 = pl.multiple_of(qp * 128, 128)
        for tt in range(4):
            h0 = pl.multiple_of((g * 8 + 2 * tt) * DH, 2 * DH)
            vh = vT_s[pl.ds(h0, 2 * DH), pl.ds(q0, WIN + QB)]
            oTs = []
            for e in range(2):
                c0 = (e * 4 + tt) * 128
                p = jnp.exp2(s_buf[:, c0:c0 + 128] - m_buf[:, c0:c0 + 128])
                l = jnp.sum(p, axis=0, keepdims=True)
                oTs.append(jnp.dot(vh[:, e * QB:e * QB + WIN], p.astype(bf16), preferred_element_type=f32) / l)
                yield
            low = lane16 < QB
            oT_s[pl.ds(h0, DH), pl.ds(q0, 128)] = jnp.where(low, oTs[0][0:DH], pltpu.roll(oTs[1][0:DH], QB, 1)).astype(bf16)
            oT_s[pl.ds(h0 + DH, DH), pl.ds(q0, 128)] = jnp.where(low, pltpu.roll(oTs[0][DH:2 * DH], QB, 1), oTs[1][DH:2 * DH]).astype(bf16)

    def attn_pair_g(i, full_mask=False):
        t0 = 2 * i
        yield from qk_g(t0 + 1, sB, mB, full_mask)
        yield from sm_g(t0, sA, mA)
        yield from qk_g(jnp.minimum(t0 + 2, NSTEP - 1), sA, mA, full_mask)
        yield from sm_g(t0 + 1, sB, mB)

    drain(qk_g(0, sA, mA, True))

    def loopA(full_mask):
        def body(i, carry):
            interleave((attn_pair_g(i, full_mask), 1), (chain(vpu_g(2 * i), vpu_g(2 * i + 1)), VW))
            return carry
        return body
    lax.fori_loop(0, 4, loopA(True), 0)
    lax.fori_loop(4, 16, loopA(False), 0)

    def loopB(i, carry):
        interleave((attn_pair_g(i), 3), (chain(*[inv_g(4 * (i - 16) + q) for q in range(4)]), 1))
        return carry
    lax.fori_loop(16, 24, loopB, 0)

    def loopC(i, carry):
        interleave((attn_pair_g(i), 1), (chain(*[fin_g(8 * (i - 24) + q) for q in range(8)]), 1))
        return carry
    lax.fori_loop(24, 32, loopC, 0)

    cp_ob = pltpu.make_async_copy(o_ref.at[:, D:2 * D], out_hbm.at[:, D:2 * D], osem.at[S // CH])
    cp_ob.start()
    cp_o.wait()

    def outp(c, carry):
        r0 = pl.multiple_of(c * CH, CH)
        o = oT_s[:, pl.ds(r0, CH)].T
        o_ref[pl.ds(r0, CH), 0:D] = jnp.dot(o, wo_ref[...], preferred_element_type=f32).astype(o_ref.dtype)
        pltpu.make_async_copy(o_ref.at[pl.ds(r0, CH), 0:D], out_hbm.at[pl.ds(r0, CH), 0:D], osem.at[c]).start()
        return carry
    lax.fori_loop(0, S // CH, outp, 0)
    cp_ob.wait()
    for c in range(S // CH):
        pltpu.make_async_copy(o_ref.at[pl.ds(c * CH, CH), 0:D], out_hbm.at[pl.ds(c * CH, CH), 0:D], osem.at[c]).wait()


KW = 8
VW = 7


@jax.jit
def pallas_concat_heads__sliding_block__ssm_conv_s4__prompt_kernel(
    A_x: jax.Array,
    A_wqkv: jax.Array,
    A_wo: jax.Array,
    B_u: jax.Array,
    B_A_re: jax.Array,
    B_A_im: jax.Array,
    B_B_re: jax.Array,
    B_B_im: jax.Array,
    B_C_re: jax.Array,
    B_C_im: jax.Array,
    B_log_dt: jax.Array,
    B_Dskip: jax.Array,
):
    out = pl.pallas_call(
        fused_kernel,
        out_shape=jax.ShapeDtypeStruct((S, 2 * D), bf16),
        in_specs=[pl.BlockSpec(memory_space=pl.ANY)] * 4 + [pl.BlockSpec(memory_space=pltpu.VMEM)] * 8,
        out_specs=pl.BlockSpec(memory_space=pl.ANY),
        scratch_shapes=[
            pltpu.VMEM((S, D), bf16),
            pltpu.VMEM((D, 3 * D), bf16),
            pltpu.VMEM((D, D), bf16),
            pltpu.VMEM((L, D), bf16),
            pltpu.VMEM((S, 2 * D), bf16),
            pltpu.SemaphoreType.DMA((4,)),
            pltpu.SemaphoreType.DMA((S // CH + 1,)),
            pltpu.VMEM((4, S, 128), bf16),
            pltpu.VMEM((4, S + W, 128), bf16),
            pltpu.VMEM((D, S + W), bf16),
            pltpu.VMEM((D, S), bf16),
            pltpu.VMEM((5, WIN, 128), f32),
            pltpu.VMEM((WIN, 16 * QB), f32),
            pltpu.VMEM((WIN, 16 * QB), f32),
            pltpu.VMEM((1, 16 * QB), f32),
            pltpu.VMEM((1, 16 * QB), f32),
            pltpu.VMEM((D, D), bf16),
            pltpu.VMEM((18, D, NM), f32),
            pltpu.VMEM((40 * 256, 128), f32),
            pltpu.VMEM((4 * L, 128), f32),
            pltpu.VMEM((32 * 128, 256), bf16),
            pltpu.VMEM((32, 256, 256), f32),
            pltpu.VMEM((32, 256, 256), f32),
            pltpu.VMEM((4 * L, 128), f32),
            pltpu.VMEM((64, 128), f32),
            pltpu.VMEM((32 * 256, 128), bf16),
        ],
        compiler_params=pltpu.CompilerParams(vmem_limit_bytes=110 * 1024 * 1024),
    )(A_x[0], A_wqkv, A_wo, B_u[0], B_A_re, B_A_im, B_B_re, B_B_im, B_C_re, B_C_im, B_log_dt, B_Dskip)
    return out[None]
```

```python
import math
import cmath
import jax
import jax.numpy as jnp
from jax import lax
import jax.experimental.pallas as pl
import jax.experimental.pallas.tpu as pltpu

f32 = jnp.float32
bf16 = jnp.bfloat16
NT = (((1,), (1,)), ((), ()))

S, D, H, DH, W = 2048, 512, 32, 16, 256
QB = 64
WIN = QB + W
NSTEP = (S // 128) * 4
CH = 256
QSCALE = 0.25 * 1.4426950408889634
L, NM = 2048, 128


def interleave(*streams):
    active = [[g, w] for g, w in streams]
    while active:
        for item in list(active):
            g, w = item
            for _ in range(w):
                try:
                    next(g)
                except StopIteration:
                    active.remove(item)
                    break


def drain(g):
    for _ in g:
        pass


def chain(*gens):
    for g in gens:
        yield from g


def sincos(x):
    kf = jnp.floor(x * 0.6366197723675814 + 0.5)
    r = x - kf * 1.5703125
    r = r - kf * 4.837512969970703125e-4
    r = r - kf * 7.54978995489188216e-8
    q = kf.astype(jnp.int32) & 3
    r2 = r * r
    s = r + r * r2 * (-1.6666654611e-1 + r2 * (8.3321608736e-3 + r2 * (-1.9515295891e-4)))
    c = 1.0 - 0.5 * r2 + r2 * r2 * (4.166664568298827e-2 + r2 * (-1.388731625493765e-3 + r2 * 2.443315711809948e-5))
    swap = (q & 1) == 1
    sn = jnp.where(swap, c, s)
    cs = jnp.where(swap, s, c)
    sn = jnp.where(q >= 2, -sn, sn)
    cs = jnp.where((q == 1) | (q == 2), -cs, cs)
    return sn, cs


def cexp(zr, zi):
    e = jnp.exp(zr)
    s, c = sincos(zi)
    return e * c, e * s


def cmul(ar, ai, br, bi):
    return ar * br - ai * bi, ar * bi + ai * br


def csq(ar, ai):
    return ar * ar - ai * ai, 2.0 * ar * ai


def cmulc(a, w):
    ar, ai = a
    if abs(w - 1) < 1e-12:
        return a
    if abs(w + 1) < 1e-12:
        return (-ar, -ai)
    if abs(w + 1j) < 1e-12:
        return (ai, -ar)
    if abs(w - 1j) < 1e-12:
        return (-ai, ar)
    wr, wi = float(w.real), float(w.imag)
    return (ar * wr - ai * wi, ar * wi + ai * wr)


def fft_g(x, sign):
    n = len(x)
    bits = n.bit_length() - 1
    a = [x[int(format(i, '0%db' % bits)[::-1], 2)] for i in range(n)]
    size = 2
    while size <= n:
        half = size // 2
        for start in range(0, n, size):
            for k in range(half):
                t = cmulc(a[start + k + half], cmath.exp(sign * 2j * math.pi * k / size))
                u = a[start + k]
                a[start + k] = (u[0] + t[0], u[1] + t[1])
                a[start + k + half] = (u[0] - t[0], u[1] - t[1])
        yield
        size *= 2
    return a


def fused_kernel(x_hbm, wqkv_hbm, wo_hbm, u_hbm, are_ref, aim_ref, bre_ref, bim_ref, cre_ref, cim_ref, ldt_ref, dsk_in,
                 out_hbm,
                 x_ref, wqkv_ref, wo_ref, u_ref, o_ref, isem, osem,
                 q_s, k_s, vT_s, oT_s, mask_s, sA, sB, mA, mB, wvT_s,
                 par, R, uf, Wf, PU, PK, yf, tw, SU):
    def cp_x(c):
        return pltpu.make_async_copy(x_hbm.at[pl.ds(c * CH, CH), :], x_ref.at[pl.ds(c * CH, CH), :], isem.at[3 + c])
    cp_w = pltpu.make_async_copy(wqkv_hbm, wqkv_ref, isem.at[0])
    cp_u = pltpu.make_async_copy(u_hbm, u_ref, isem.at[1])
    cp_o = pltpu.make_async_copy(wo_hbm, wo_ref, isem.at[2])
    cp_w.start()
    for c in range(S // CH):
        cp_x(c).start()
    cp_u.start(); cp_o.start()
    dsk_row = dsk_in[...].reshape(1, D)

    dt = jnp.exp(ldt_ref[...].astype(f32)).astype(bf16).astype(f32).reshape(1, D)
    dt = jnp.broadcast_to(dt, (NM, D)).T
    zr = are_ref[...].astype(f32) * dt
    zi = aim_ref[...].astype(f32) * dt
    cr, ci = cmul(cre_ref[...].astype(f32), cim_ref[...].astype(f32),
                  bre_ref[...].astype(f32) * dt, bim_ref[...].astype(f32) * dt)
    par[0] = cr
    par[1] = ci
    a1 = cexp(zr, zi)
    a2 = csq(*a1)
    par[2] = a1[0]; par[3] = a1[1]
    par[4] = a2[0]; par[5] = a2[1]
    a4 = csq(*a2)
    par[6] = a4[0]; par[7] = a4[1]
    a8 = csq(*a4)
    par[8] = a8[0]; par[9] = a8[1]
    a32 = cexp(zr * 32, -zi * 32)
    par[10] = a32[0]; par[11] = a32[1]
    a64 = csq(*a32)
    par[12] = a64[0]; par[13] = a64[1]
    a128 = csq(*a64)
    par[14] = a128[0]; par[15] = a128[1]
    a256 = csq(*a128)
    par[16] = a256[0]; par[17] = a256[1]

    rr = lax.broadcasted_iota(jnp.int32, (128, 128), 0)
    cc = lax.broadcasted_iota(jnp.int32, (128, 128), 1)
    same = (rr >= 64) == (cc >= 64)
    nA = ((rr & 63) * (2 * (cc & 63) + 1)) & 255
    sA_, cA_ = sincos(nA.astype(f32) * (2.0 * math.pi / 256))
    Ar = jnp.where(same, cA_, 0.0)
    Ai = jnp.where(same, -sA_, 0.0)
    jb = lax.broadcasted_iota(jnp.int32, (32, 128), 0)
    kb = lax.broadcasted_iota(jnp.int32, (32, 128), 1) & 63
    sB_, cB_ = sincos((jb * (2 * kb + 1)).astype(f32) * (2.0 * math.pi / 8192))
    tw[0:32, :] = cB_
    tw[32:64, :] = -sB_

    def wgen(j, carry):
        wr, wi = cmul(Ar, Ai, tw[pl.ds(j, 1), :], tw[pl.ds(32 + j, 1), :])
        Wf[pl.ds(pl.multiple_of(j * 128, 128), 128), :] = jnp.concatenate([wr, wi], 1).astype(bf16)
        return carry
    lax.fori_loop(0, 32, wgen, 0)

    rI = lax.broadcasted_iota(jnp.int32, (WIN, 128), 0)
    cq = lax.broadcasted_iota(jnp.int32, (WIN, 128), 1) & (QB - 1)
    for v in range(5):
        valid = (rI > cq) & (rI - W <= cq) & (rI >= W - v * QB)
        mask_s[v] = jnp.where(valid, 0.0, -1e9).astype(f32)
    for b in range(4):
        k_s[b, 0:W, :] = jnp.zeros((W, 128), bf16)
    vT_s[:, 0:W] = jnp.zeros((D, W), bf16)
    cp_w.wait()
    wvT_s[...] = wqkv_ref[:, 2 * D:3 * D].T

    sub = lax.broadcasted_iota(jnp.int32, (8, NM), 0)
    b0 = (sub & 1) == 1
    b1 = (sub & 2) == 2
    b2 = (sub & 4) == 4
    lane40 = lax.broadcasted_iota(jnp.int32, (40, 128), 1)

    def row(k, d):
        return par[k, pl.ds(d, 1), :]

    def pow8(d, k0):
        f0 = (jnp.where(b0, row(k0, d), 1.0), jnp.where(b0, row(k0 + 1, d), 0.0))
        f1 = (jnp.where(b1, row(k0 + 2, d), 1.0), jnp.where(b1, row(k0 + 3, d), 0.0))
        f2 = (jnp.where(b2, row(k0 + 4, d), 1.0), jnp.where(b2, row(k0 + 5, d), 0.0))
        return cmul(*cmul(*f0, *f1), *f2)

    def chan_g(d):
        T = cmul(row(0, d), row(1, d), *pow8(d, 2))
        Tr, Ti = [T[0]], [T[1]]
        yield
        for _ in range(4):
            T = cmul(*T, row(8, d), row(9, d))
            Tr.append(T[0]); Ti.append(T[1])
        yield
        P = pow8(d, 10)
        Pr, Pi = [P[0]], [P[1]]
        yield
        for it in range(7):
            P = cmul(*P, row(16, d), row(17, d))
            Pr.append(P[0]); Pi.append(P[1])
            if it == 3:
                yield
        yield
        lhs = jnp.concatenate([jnp.concatenate(Tr, 0), jnp.concatenate(Ti, 0)], 1)
        rhs = jnp.concatenate([jnp.concatenate(Pr, 0), jnp.concatenate(Pi, 0)], 1)
        return lhs, rhs

    def kgen_pair_g(c):
        l0, r0 = yield from chan_g(c)
        l1, r1 = yield from chan_g(c + 256)
        lhs = jnp.concatenate([l0, l1], 0).astype(bf16)
        rhs = jnp.concatenate([r0, r1], 0).astype(bf16)
        out = lax.dot_general(lhs, rhs, NT, preferred_element_type=f32)
        R[pl.ds(c, 40, stride=256), :] = jnp.where(lane40 < 64, out[0:40], out[40:80])
        yield

    def ugather_g(j):
        for beta in range(2):
            blk = jnp.concatenate([uf[pl.ds(beta * L + j, 64, stride=32), :],
                                   uf[pl.ds((2 + beta) * L + j, 64, stride=32), :]], 0)
            yield
            SU[pl.ds(pl.multiple_of(j * 256 + beta * 128, 128), 128), :] = blk.T.astype(bf16)
            yield

    def proj_g(c):
        r0 = pl.multiple_of(c * CH, CH)
        for mh in range(CH // 128):
            xr = pl.ds(pl.multiple_of(r0 + mh * 128, 128), 128)
            kr = pl.ds(pl.multiple_of(W + r0 + mh * 128, 128), 128)
            for n in range(8):
                y = jnp.dot(x_ref[xr, :], wqkv_ref[:, n * 128:(n + 1) * 128], preferred_element_type=f32)
                if n < 4:
                    q_s[n, xr, :] = (y * QSCALE).astype(bf16)
                else:
                    k_s[n - 4, kr, :] = y.astype(bf16)
                yield
            for m in range(4):
                vT = lax.dot_general(wvT_s[m * 128:(m + 1) * 128, :], x_ref[xr, :], NT, preferred_element_type=f32)
                vT_s[m * 128:(m + 1) * 128, kr] = vT.astype(bf16)
                yield

    NPI = 256 // (S // CH)

    def kgen_proj(it, carry):
        kg = chain(*[kgen_pair_g(it * NPI + p) for p in range(NPI)])
        cp_x(it).wait()
        interleave((proj_g(it), 1), (kg, KW))
        return carry
    lax.fori_loop(0, S // CH, kgen_proj, 0)

    cp_u.wait()
    for b in range(4):
        uf[pl.ds(b * L, L), :] = u_ref[:, b * 128:(b + 1) * 128].astype(f32)

    li = lax.broadcasted_iota(jnp.int32, (256, 128), 1) & 63

    def fwd(j, carry):
        def slab(s):
            t = j if s == 0 else ((j + (1 << (s - 1)) - 1 + ((j >> s) & 1)) >> s) << s
            return R[pl.ds(pl.multiple_of(t * 256, 256), 256), :]
        Sk = jnp.where(li < 8, slab(0), jnp.where(li < 16, slab(1), jnp.where(li < 32, slab(2), slab(3)))).astype(bf16)
        drain(ugather_g(j))
        Su = SU[pl.ds(pl.multiple_of(j * 256, 256), 256), :]
        P = jnp.dot(jnp.concatenate([Su, Sk], 0), Wf[pl.ds(pl.multiple_of(j * 128, 128), 128), :],
                    preferred_element_type=f32)
        PU[j] = P[0:256]
        PK[j] = P[256:512]
        return carry
    lax.fori_loop(0, 32, fwd, 0, unroll=4)

    def ld(ref, slot, r0):
        return (ref[slot, pl.ds(r0, 8), 0:128], ref[slot, pl.ds(r0, 8), 128:256])

    def st(ref, slot, r0, v):
        ref[slot, pl.ds(r0, 8), 0:128] = v[0]
        ref[slot, pl.ds(r0, 8), 128:256] = v[1]

    def vpu_g(ch):
        r0 = pl.multiple_of(ch * 8, 8)
        for ref in (PU, PK):
            for j0 in range(4):
                a = yield from fft_g([ld(ref, 4 * j1 + j0, r0) for j1 in range(8)], -1)
                for k0 in range(8):
                    st(ref, 4 * k0 + j0, r0, cmulc(a[k0], cmath.exp(-2j * math.pi * j0 * k0 / 32)))
                yield
        for k0 in range(8):
            xu = yield from fft_g([ld(PU, 4 * k0 + j0, r0) for j0 in range(4)], -1)
            xk = yield from fft_g([ld(PK, 4 * k0 + j0, r0) for j0 in range(4)], -1)
            y = [cmul(*xu[k1], *xk[k1]) for k1 in range(4)]
            bb = yield from fft_g(y, +1)
            for j0 in range(4):
                st(PU, 4 * k0 + j0, r0, cmulc(bb[j0], cmath.exp(2j * math.pi * j0 * k0 / 32)))
            yield
        for j0 in range(4):
            z = yield from fft_g([ld(PU, 4 * k0 + j0, r0) for k0 in range(8)], +1)
            for j1 in range(8):
                st(PU, 4 * j1 + j0, r0, z[j1])
            yield

    def inv_g(j):
        Z = PU[j].astype(bf16)
        O = lax.dot_general(Z, Wf[pl.ds(pl.multiple_of(j * 128, 128), 128), :], NT,
                            preferred_element_type=f32) * (2.0 / 4096)
        yield
        j64 = pl.multiple_of(j * 64, 64)
        for beta in range(2):
            T = O[beta * 128:(beta + 1) * 128, :].T
            yf[pl.ds(beta * L + j64, 64), :] = T[0:64]
            yf[pl.ds((2 + beta) * L + j64, 64), :] = T[64:128]
            yield

    def fin_g(i):
        r0 = pl.multiple_of(i * 32, 32)
        for b in range(4):
            yb = yf[pl.ds(b * L + i, 32, stride=64), :].astype(bf16)
            ub = u_ref[pl.ds(r0, 32), b * 128:(b + 1) * 128]
            o_ref[pl.ds(r0, 32), D + b * 128:D + (b + 1) * 128] = yb + ub * dsk_row[:, b * 128:(b + 1) * 128]
            yield

    lane_head = lax.broadcasted_iota(jnp.int32, (QB // 2, 128), 1) // DH
    lane16 = lax.broadcasted_iota(jnp.int32, (DH, 128), 1)

    def qk_g(t, s_buf, m_buf, full_mask):
        qp = t // 4
        g = t % 4
        q0 = pl.multiple_of(qp * 128, 128)
        kg = k_s[g, pl.ds(q0, WIN + QB), :]
        for e in range(2):
            qg = pltpu.bitcast(q_s[g, pl.ds(q0 + e * QB, QB), :], jnp.uint32)
            qm = jnp.concatenate([pltpu.bitcast(jnp.where(lane_head == hh, qg, jnp.uint32(0)), bf16) for hh in range(8)], axis=0)
            sT_all = lax.dot_general(kg[e * QB:e * QB + WIN], qm, NT, preferred_element_type=f32)
            if full_mask:
                bias = mask_s[jnp.minimum(2 * qp + e, 4)]
            yield
            for tt in range(4):
                c0 = (e * 4 + tt) * 128
                if full_mask:
                    sT = sT_all[:, tt * 128:(tt + 1) * 128] + bias
                else:
                    sT = jnp.concatenate([sT_all[0:QB, tt * 128:(tt + 1) * 128] + mask_s[4, 0:QB, :],
                                          sT_all[QB:W, tt * 128:(tt + 1) * 128],
                                          sT_all[W:WIN, tt * 128:(tt + 1) * 128] + mask_s[4, W:WIN, :]], axis=0)
                m_buf[:, c0:c0 + 128] = jnp.max(sT, axis=0, keepdims=True)
                s_buf[:, c0:c0 + 128] = sT
                yield

    def sm_g(t, s_buf, m_buf):
        qp = t // 4
        g = t % 4
        q0 = pl.multiple_of(qp * 128, 128)
        for tt in range(4):
            h0 = pl.multiple_of((g * 8 + 2 * tt) * DH, 2 * DH)
            vh = vT_s[pl.ds(h0, 2 * DH), pl.ds(q0, WIN + QB)]
            oTs = []
            for e in range(2):
                c0 = (e * 4 + tt) * 128
                p = jnp.exp2(s_buf[:, c0:c0 + 128] - m_buf[:, c0:c0 + 128])
                l = jnp.sum(p, axis=0, keepdims=True)
                oTs.append(jnp.dot(vh[:, e * QB:e * QB + WIN], p.astype(bf16), preferred_element_type=f32) / l)
                yield
            low = lane16 < QB
            oT_s[pl.ds(h0, DH), pl.ds(q0, 128)] = jnp.where(low, oTs[0][0:DH], pltpu.roll(oTs[1][0:DH], QB, 1)).astype(bf16)
            oT_s[pl.ds(h0 + DH, DH), pl.ds(q0, 128)] = jnp.where(low, pltpu.roll(oTs[0][DH:2 * DH], QB, 1), oTs[1][DH:2 * DH]).astype(bf16)

    def attn_quad_g(i, full_mask=False):
        for half in range(2):
            t0 = 4 * i + 2 * half
            yield from qk_g(t0 + 1, sB, mB, full_mask)
            yield from sm_g(t0, sA, mA)
            yield from qk_g(jnp.minimum(t0 + 2, NSTEP - 1), sA, mA, full_mask)
            yield from sm_g(t0 + 1, sB, mB)

    drain(qk_g(0, sA, mA, True))

    def loopA(full_mask):
        def body(i, carry):
            interleave((attn_quad_g(i, full_mask), 1), (chain(*[vpu_g(4 * i + q) for q in range(4)]), VW))
            return carry
        return body
    lax.fori_loop(0, 2, loopA(True), 0)
    lax.fori_loop(2, 8, loopA(False), 0)

    def loopB(i, carry):
        interleave((attn_quad_g(i), 3), (chain(*[inv_g(8 * (i - 8) + q) for q in range(8)]), 1))
        return carry
    lax.fori_loop(8, 12, loopB, 0)

    def loopC(i, carry):
        interleave((attn_quad_g(i), 1), (chain(*[fin_g(16 * (i - 12) + q) for q in range(16)]), 1))
        return carry
    lax.fori_loop(12, 16, loopC, 0)

    cp_ob = pltpu.make_async_copy(o_ref.at[:, D:2 * D], out_hbm.at[:, D:2 * D], osem.at[S // CH])
    cp_ob.start()
    cp_o.wait()

    def outp(c, carry):
        r0 = pl.multiple_of(c * CH, CH)
        o = oT_s[:, pl.ds(r0, CH)].T
        o_ref[pl.ds(r0, CH), 0:D] = jnp.dot(o, wo_ref[...], preferred_element_type=f32).astype(o_ref.dtype)
        pltpu.make_async_copy(o_ref.at[pl.ds(r0, CH), 0:D], out_hbm.at[pl.ds(r0, CH), 0:D], osem.at[c]).start()
        return carry
    lax.fori_loop(0, S // CH, outp, 0)
    cp_ob.wait()
    for c in range(S // CH):
        pltpu.make_async_copy(o_ref.at[pl.ds(c * CH, CH), 0:D], out_hbm.at[pl.ds(c * CH, CH), 0:D], osem.at[c]).wait()


KW = 8
VW = 7


@jax.jit
def pallas_concat_heads__sliding_block__ssm_conv_s4__prompt_kernel(
    A_x: jax.Array,
    A_wqkv: jax.Array,
    A_wo: jax.Array,
    B_u: jax.Array,
    B_A_re: jax.Array,
    B_A_im: jax.Array,
    B_B_re: jax.Array,
    B_B_im: jax.Array,
    B_C_re: jax.Array,
    B_C_im: jax.Array,
    B_log_dt: jax.Array,
    B_Dskip: jax.Array,
):
    out = pl.pallas_call(
        fused_kernel,
        out_shape=jax.ShapeDtypeStruct((S, 2 * D), bf16),
        in_specs=[pl.BlockSpec(memory_space=pl.ANY)] * 4 + [pl.BlockSpec(memory_space=pltpu.VMEM)] * 8,
        out_specs=pl.BlockSpec(memory_space=pl.ANY),
        scratch_shapes=[
            pltpu.VMEM((S, D), bf16),
            pltpu.VMEM((D, 3 * D), bf16),
            pltpu.VMEM((D, D), bf16),
            pltpu.VMEM((L, D), bf16),
            pltpu.VMEM((S, 2 * D), bf16),
            pltpu.SemaphoreType.DMA((3 + S // CH,)),
            pltpu.SemaphoreType.DMA((S // CH + 1,)),
            pltpu.VMEM((4, S, 128), bf16),
            pltpu.VMEM((4, S + W, 128), bf16),
            pltpu.VMEM((D, S + W), bf16),
            pltpu.VMEM((D, S), bf16),
            pltpu.VMEM((5, WIN, 128), f32),
            pltpu.VMEM((WIN, 16 * QB), f32),
            pltpu.VMEM((WIN, 16 * QB), f32),
            pltpu.VMEM((1, 16 * QB), f32),
            pltpu.VMEM((1, 16 * QB), f32),
            pltpu.VMEM((D, D), bf16),
            pltpu.VMEM((18, D, NM), f32),
            pltpu.VMEM((40 * 256, 128), f32),
            pltpu.VMEM((4 * L, 128), f32),
            pltpu.VMEM((32 * 128, 256), bf16),
            pltpu.VMEM((32, 256, 256), f32),
            pltpu.VMEM((32, 256, 256), f32),
            pltpu.VMEM((4 * L, 128), f32),
            pltpu.VMEM((64, 128), f32),
            pltpu.VMEM((32 * 256, 128), bf16),
        ],
        compiler_params=pltpu.CompilerParams(vmem_limit_bytes=110 * 1024 * 1024),
    )(A_x[0], A_wqkv, A_wo, B_u[0], B_A_re, B_A_im, B_B_re, B_B_im, B_C_re, B_C_im, B_log_dt, B_Dskip)
    return out[None]
```

```python
import math
import cmath
import jax
import jax.numpy as jnp
from jax import lax
import jax.experimental.pallas as pl
import jax.experimental.pallas.tpu as pltpu

f32 = jnp.float32
bf16 = jnp.bfloat16
NT = (((1,), (1,)), ((), ()))

S, D, H, DH, W = 2048, 512, 32, 16, 256
QB = 64
WIN = QB + W
NSTEP = (S // 128) * 4
CH = 256
QSCALE = 0.25 * 1.4426950408889634
L, NM = 2048, 128


def interleave(*streams):
    active = [[g, w] for g, w in streams]
    while active:
        for item in list(active):
            g, w = item
            for _ in range(w):
                try:
                    next(g)
                except StopIteration:
                    active.remove(item)
                    break


def drain(g):
    for _ in g:
        pass


def chain(*gens):
    for g in gens:
        yield from g


def sincos(x):
    kf = jnp.floor(x * 0.6366197723675814 + 0.5)
    r = x - kf * 1.5703125
    r = r - kf * 4.837512969970703125e-4
    r = r - kf * 7.54978995489188216e-8
    q = kf.astype(jnp.int32) & 3
    r2 = r * r
    s = r + r * r2 * (-1.6666654611e-1 + r2 * (8.3321608736e-3 + r2 * (-1.9515295891e-4)))
    c = 1.0 - 0.5 * r2 + r2 * r2 * (4.166664568298827e-2 + r2 * (-1.388731625493765e-3 + r2 * 2.443315711809948e-5))
    swap = (q & 1) == 1
    sn = jnp.where(swap, c, s)
    cs = jnp.where(swap, s, c)
    sn = jnp.where(q >= 2, -sn, sn)
    cs = jnp.where((q == 1) | (q == 2), -cs, cs)
    return sn, cs


def cexp(zr, zi):
    e = jnp.exp(zr)
    s, c = sincos(zi)
    return e * c, e * s


def cmul(ar, ai, br, bi):
    return ar * br - ai * bi, ar * bi + ai * br


def csq(ar, ai):
    return ar * ar - ai * ai, 2.0 * ar * ai


def cmulc(a, w):
    ar, ai = a
    if abs(w - 1) < 1e-12:
        return a
    if abs(w + 1) < 1e-12:
        return (-ar, -ai)
    if abs(w + 1j) < 1e-12:
        return (ai, -ar)
    if abs(w - 1j) < 1e-12:
        return (-ai, ar)
    wr, wi = float(w.real), float(w.imag)
    return (ar * wr - ai * wi, ar * wi + ai * wr)


def fft_g(x, sign):
    n = len(x)
    bits = n.bit_length() - 1
    a = [x[int(format(i, '0%db' % bits)[::-1], 2)] for i in range(n)]
    size = 2
    while size <= n:
        half = size // 2
        for start in range(0, n, size):
            for k in range(half):
                t = cmulc(a[start + k + half], cmath.exp(sign * 2j * math.pi * k / size))
                u = a[start + k]
                a[start + k] = (u[0] + t[0], u[1] + t[1])
                a[start + k + half] = (u[0] - t[0], u[1] - t[1])
        yield
        size *= 2
    return a


def fused_kernel(x_hbm, wqkv_hbm, wo_hbm, u_hbm, are_ref, aim_ref, bre_ref, bim_ref, cre_ref, cim_ref, ldt_ref, dsk_in,
                 out_hbm,
                 x_ref, wqkv_ref, wo_ref, u_ref, o_ref, isem, osem,
                 q_s, k_s, vT_s, oT_s, mask_s, sA, sB, mA, mB, wvT_s,
                 par, R, uf, Wf, PU, PK, yf, tw, SU):
    def cp_x(c):
        return pltpu.make_async_copy(x_hbm.at[pl.ds(c * CH, CH), :], x_ref.at[pl.ds(c * CH, CH), :], isem.at[3 + c])
    cp_w = pltpu.make_async_copy(wqkv_hbm, wqkv_ref, isem.at[0])
    cp_u = pltpu.make_async_copy(u_hbm, u_ref, isem.at[1])
    cp_o = pltpu.make_async_copy(wo_hbm, wo_ref, isem.at[2])
    cp_w.start()
    for c in range(S // CH):
        cp_x(c).start()
    cp_u.start(); cp_o.start()
    dsk_row = dsk_in[...].reshape(1, D)

    dt = jnp.exp(ldt_ref[...].astype(f32)).astype(bf16).astype(f32).reshape(1, D)
    dt = jnp.broadcast_to(dt, (NM, D)).T
    zr = are_ref[...].astype(f32) * dt
    zi = aim_ref[...].astype(f32) * dt
    cr, ci = cmul(cre_ref[...].astype(f32), cim_ref[...].astype(f32),
                  bre_ref[...].astype(f32) * dt, bim_ref[...].astype(f32) * dt)
    par[0] = cr
    par[1] = ci
    a1 = cexp(zr, zi)
    a2 = csq(*a1)
    par[2] = a1[0]; par[3] = a1[1]
    par[4] = a2[0]; par[5] = a2[1]
    a4 = csq(*a2)
    par[6] = a4[0]; par[7] = a4[1]
    a8 = csq(*a4)
    par[8] = a8[0]; par[9] = a8[1]
    a32 = cexp(zr * 32, -zi * 32)
    par[10] = a32[0]; par[11] = a32[1]
    a64 = csq(*a32)
    par[12] = a64[0]; par[13] = a64[1]
    a128 = csq(*a64)
    par[14] = a128[0]; par[15] = a128[1]
    a256 = csq(*a128)
    par[16] = a256[0]; par[17] = a256[1]

    rr = lax.broadcasted_iota(jnp.int32, (128, 128), 0)
    cc = lax.broadcasted_iota(jnp.int32, (128, 128), 1)
    same = (rr >= 64) == (cc >= 64)
    nA = ((rr & 63) * (2 * (cc & 63) + 1)) & 255
    sA_, cA_ = sincos(nA.astype(f32) * (2.0 * math.pi / 256))
    Ar = jnp.where(same, cA_, 0.0)
    Ai = jnp.where(same, -sA_, 0.0)
    jb = lax.broadcasted_iota(jnp.int32, (32, 128), 0)
    kb = lax.broadcasted_iota(jnp.int32, (32, 128), 1) & 63
    sB_, cB_ = sincos((jb * (2 * kb + 1)).astype(f32) * (2.0 * math.pi / 8192))
    tw[0:32, :] = cB_
    tw[32:64, :] = -sB_

    def wgen(j, carry):
        wr, wi = cmul(Ar, Ai, tw[pl.ds(j, 1), :], tw[pl.ds(32 + j, 1), :])
        Wf[pl.ds(pl.multiple_of(j * 128, 128), 128), :] = jnp.concatenate([wr, wi], 1).astype(bf16)
        return carry
    lax.fori_loop(0, 32, wgen, 0)

    rI = lax.broadcasted_iota(jnp.int32, (WIN, 128), 0)
    cq = lax.broadcasted_iota(jnp.int32, (WIN, 128), 1) & (QB - 1)
    for v in range(5):
        valid = (rI > cq) & (rI - W <= cq) & (rI >= W - v * QB)
        mask_s[v] = jnp.where(valid, 0.0, -1e9).astype(f32)
    for b in range(4):
        k_s[b, 0:W, :] = jnp.zeros((W, 128), bf16)
    vT_s[:, 0:W] = jnp.zeros((D, W), bf16)
    cp_w.wait()
    wvT_s[...] = wqkv_ref[:, 2 * D:3 * D].T

    sub = lax.broadcasted_iota(jnp.int32, (8, NM), 0)
    b0 = (sub & 1) == 1
    b1 = (sub & 2) == 2
    b2 = (sub & 4) == 4
    lane40 = lax.broadcasted_iota(jnp.int32, (40, 128), 1)

    def row(k, d):
        return par[k, pl.ds(d, 1), :]

    def pow8(d, k0):
        f0 = (jnp.where(b0, row(k0, d), 1.0), jnp.where(b0, row(k0 + 1, d), 0.0))
        f1 = (jnp.where(b1, row(k0 + 2, d), 1.0), jnp.where(b1, row(k0 + 3, d), 0.0))
        f2 = (jnp.where(b2, row(k0 + 4, d), 1.0), jnp.where(b2, row(k0 + 5, d), 0.0))
        return cmul(*cmul(*f0, *f1), *f2)

    def chan_g(d):
        T = cmul(row(0, d), row(1, d), *pow8(d, 2))
        Tr, Ti = [T[0]], [T[1]]
        yield
        for _ in range(4):
            T = cmul(*T, row(8, d), row(9, d))
            Tr.append(T[0]); Ti.append(T[1])
        yield
        P = pow8(d, 10)
        Pr, Pi = [P[0]], [P[1]]
        yield
        for it in range(7):
            P = cmul(*P, row(16, d), row(17, d))
            Pr.append(P[0]); Pi.append(P[1])
            if it == 3:
                yield
        yield
        lhs = jnp.concatenate([jnp.concatenate(Tr, 0), jnp.concatenate(Ti, 0)], 1)
        rhs = jnp.concatenate([jnp.concatenate(Pr, 0), jnp.concatenate(Pi, 0)], 1)
        return lhs, rhs

    def kgen_pair_g(c):
        l0, r0 = yield from chan_g(c)
        l1, r1 = yield from chan_g(c + 256)
        lhs = jnp.concatenate([l0, l1], 0).astype(bf16)
        rhs = jnp.concatenate([r0, r1], 0).astype(bf16)
        out = lax.dot_general(lhs, rhs, NT, preferred_element_type=f32)
        R[pl.ds(c, 40, stride=256), :] = jnp.where(lane40 < 64, out[0:40], out[40:80])
        yield

    def ugather_g(j):
        for beta in range(2):
            blk = jnp.concatenate([uf[pl.ds(beta * L + j, 64, stride=32), :],
                                   uf[pl.ds((2 + beta) * L + j, 64, stride=32), :]], 0)
            yield
            SU[pl.ds(pl.multiple_of(j * 256 + beta * 128, 128), 128), :] = blk.T.astype(bf16)
            yield

    def proj_g(c):
        r0 = pl.multiple_of(c * CH, CH)
        xr = pl.ds(r0, CH)
        kr = pl.ds(pl.multiple_of(W + r0, 128), CH)
        for n in range(8):
            y = jnp.dot(x_ref[xr, :], wqkv_ref[:, n * 128:(n + 1) * 128], preferred_element_type=f32)
            if n < 4:
                q_s[n, xr, :] = (y * QSCALE).astype(bf16)
            else:
                k_s[n - 4, kr, :] = y.astype(bf16)
            yield
        for m in range(4):
            vT = lax.dot_general(wvT_s[m * 128:(m + 1) * 128, :], x_ref[xr, :], NT, preferred_element_type=f32)
            vT_s[m * 128:(m + 1) * 128, kr] = vT.astype(bf16)
            yield

    NPI = 256 // (S // CH)

    def kgen_proj(it, carry):
        kg = chain(*[kgen_pair_g(it * NPI + p) for p in range(NPI)])
        cp_x(it).wait()
        interleave((proj_g(it), 1), (kg, KW))
        return carry
    lax.fori_loop(0, S // CH, kgen_proj, 0)

    cp_u.wait()
    for b in range(4):
        uf[pl.ds(b * L, L), :] = u_ref[:, b * 128:(b + 1) * 128].astype(f32)

    li = lax.broadcasted_iota(jnp.int32, (256, 128), 1) & 63

    def fwd(j, carry):
        def slab(s):
            t = j if s == 0 else ((j + (1 << (s - 1)) - 1 + ((j >> s) & 1)) >> s) << s
            return R[pl.ds(pl.multiple_of(t * 256, 256), 256), :]
        Sk = jnp.where(li < 8, slab(0), jnp.where(li < 16, slab(1), jnp.where(li < 32, slab(2), slab(3)))).astype(bf16)
        drain(ugather_g(j))
        Su = SU[pl.ds(pl.multiple_of(j * 256, 256), 256), :]
        P = jnp.dot(jnp.concatenate([Su, Sk], 0), Wf[pl.ds(pl.multiple_of(j * 128, 128), 128), :],
                    preferred_element_type=f32)
        PU[j] = P[0:256]
        PK[j] = P[256:512]
        return carry
    lax.fori_loop(0, 32, fwd, 0, unroll=4)

    def ld(ref, slot, r0):
        return (ref[slot, pl.ds(r0, 8), 0:128], ref[slot, pl.ds(r0, 8), 128:256])

    def st(ref, slot, r0, v):
        ref[slot, pl.ds(r0, 8), 0:128] = v[0]
        ref[slot, pl.ds(r0, 8), 128:256] = v[1]

    def vpu_g(ch):
        r0 = pl.multiple_of(ch * 8, 8)
        for ref in (PU, PK):
            for j0 in range(4):
                a = yield from fft_g([ld(ref, 4 * j1 + j0, r0) for j1 in range(8)], -1)
                for k0 in range(8):
                    st(ref, 4 * k0 + j0, r0, cmulc(a[k0], cmath.exp(-2j * math.pi * j0 * k0 / 32)))
                yield
        for k0 in range(8):
            xu = yield from fft_g([ld(PU, 4 * k0 + j0, r0) for j0 in range(4)], -1)
            xk = yield from fft_g([ld(PK, 4 * k0 + j0, r0) for j0 in range(4)], -1)
            y = [cmul(*xu[k1], *xk[k1]) for k1 in range(4)]
            bb = yield from fft_g(y, +1)
            for j0 in range(4):
                st(PU, 4 * k0 + j0, r0, cmulc(bb[j0], cmath.exp(2j * math.pi * j0 * k0 / 32)))
            yield
        for j0 in range(4):
            z = yield from fft_g([ld(PU, 4 * k0 + j0, r0) for k0 in range(8)], +1)
            for j1 in range(8):
                st(PU, 4 * j1 + j0, r0, z[j1])
            yield

    def inv_g(j):
        Z = PU[j].astype(bf16)
        O = lax.dot_general(Z, Wf[pl.ds(pl.multiple_of(j * 128, 128), 128), :], NT,
                            preferred_element_type=f32) * (2.0 / 4096)
        yield
        j64 = pl.multiple_of(j * 64, 64)
        for beta in range(2):
            T = O[beta * 128:(beta + 1) * 128, :].T
            yf[pl.ds(beta * L + j64, 64), :] = T[0:64]
            yf[pl.ds((2 + beta) * L + j64, 64), :] = T[64:128]
            yield

    def fin_g(i):
        r0 = pl.multiple_of(i * 32, 32)
        for b in range(4):
            yb = yf[pl.ds(b * L + i, 32, stride=64), :].astype(bf16)
            ub = u_ref[pl.ds(r0, 32), b * 128:(b + 1) * 128]
            o_ref[pl.ds(r0, 32), D + b * 128:D + (b + 1) * 128] = yb + ub * dsk_row[:, b * 128:(b + 1) * 128]
            yield

    lane_head = lax.broadcasted_iota(jnp.int32, (QB // 2, 128), 1) // DH
    lane16 = lax.broadcasted_iota(jnp.int32, (DH, 128), 1)

    def qk_g(t, s_buf, m_buf, full_mask):
        qp = t // 4
        g = t % 4
        q0 = pl.multiple_of(qp * 128, 128)
        kg = k_s[g, pl.ds(q0, WIN + QB), :]
        for e in range(2):
            qg = pltpu.bitcast(q_s[g, pl.ds(q0 + e * QB, QB), :], jnp.uint32)
            qm = jnp.concatenate([pltpu.bitcast(jnp.where(lane_head == hh, qg, jnp.uint32(0)), bf16) for hh in range(8)], axis=0)
            sT_all = lax.dot_general(kg[e * QB:e * QB + WIN], qm, NT, preferred_element_type=f32)
            if full_mask:
                bias = mask_s[jnp.minimum(2 * qp + e, 4)]
            yield
            for tt in range(4):
                c0 = (e * 4 + tt) * 128
                if full_mask:
                    sT = sT_all[:, tt * 128:(tt + 1) * 128] + bias
                else:
                    sT = jnp.concatenate([sT_all[0:QB, tt * 128:(tt + 1) * 128] + mask_s[4, 0:QB, :],
                                          sT_all[QB:W, tt * 128:(tt + 1) * 128],
                                          sT_all[W:WIN, tt * 128:(tt + 1) * 128] + mask_s[4, W:WIN, :]], axis=0)
                m_buf[:, c0:c0 + 128] = jnp.max(sT, axis=0, keepdims=True)
                s_buf[:, c0:c0 + 128] = sT
                yield

    def sm_g(t, s_buf, m_buf):
        qp = t // 4
        g = t % 4
        q0 = pl.multiple_of(qp * 128, 128)
        for tt in range(4):
            h0 = pl.multiple_of((g * 8 + 2 * tt) * DH, 2 * DH)
            vh = vT_s[pl.ds(h0, 2 * DH), pl.ds(q0, WIN + QB)]
            oTs = []
            for e in range(2):
                c0 = (e * 4 + tt) * 128
                p = jnp.exp2(s_buf[:, c0:c0 + 128] - m_buf[:, c0:c0 + 128])
                l = jnp.sum(p, axis=0, keepdims=True)
                oTs.append(jnp.dot(vh[:, e * QB:e * QB + WIN], p.astype(bf16), preferred_element_type=f32) / l)
                yield
            low = lane16 < QB
            oT_s[pl.ds(h0, DH), pl.ds(q0, 128)] = jnp.where(low, oTs[0][0:DH], pltpu.roll(oTs[1][0:DH], QB, 1)).astype(bf16)
            oT_s[pl.ds(h0 + DH, DH), pl.ds(q0, 128)] = jnp.where(low, pltpu.roll(oTs[0][DH:2 * DH], QB, 1), oTs[1][DH:2 * DH]).astype(bf16)

    def attn_oct_g(i, full_mask=False):
        for half in range(4):
            t0 = 8 * i + 2 * half
            yield from qk_g(t0 + 1, sB, mB, full_mask)
            yield from sm_g(t0, sA, mA)
            yield from qk_g(jnp.minimum(t0 + 2, NSTEP - 1), sA, mA, full_mask)
            yield from sm_g(t0 + 1, sB, mB)

    drain(qk_g(0, sA, mA, True))

    def loopA(full_mask):
        def body(i, carry):
            interleave((attn_oct_g(i, full_mask), 1), (chain(*[vpu_g(8 * i + q) for q in range(8)]), VW))
            return carry
        return body
    lax.fori_loop(0, 1, loopA(True), 0)
    lax.fori_loop(1, 4, loopA(False), 0)

    def loopB(i, carry):
        interleave((attn_oct_g(i), 3), (chain(*[inv_g(16 * (i - 4) + q) for q in range(16)]), 1))
        return carry
    lax.fori_loop(4, 6, loopB, 0)

    def loopC(i, carry):
        interleave((attn_oct_g(i), 1), (chain(*[fin_g(32 * (i - 6) + q) for q in range(32)]), 1))
        return carry
    lax.fori_loop(6, 8, loopC, 0)

    cp_ob = pltpu.make_async_copy(o_ref.at[:, D:2 * D], out_hbm.at[:, D:2 * D], osem.at[S // CH])
    cp_ob.start()
    cp_o.wait()

    def outp(c, carry):
        r0 = pl.multiple_of(c * CH, CH)
        o = oT_s[:, pl.ds(r0, CH)].T
        o_ref[pl.ds(r0, CH), 0:D] = jnp.dot(o, wo_ref[...], preferred_element_type=f32).astype(o_ref.dtype)
        pltpu.make_async_copy(o_ref.at[pl.ds(r0, CH), 0:D], out_hbm.at[pl.ds(r0, CH), 0:D], osem.at[c]).start()
        return carry
    lax.fori_loop(0, S // CH, outp, 0)
    cp_ob.wait()
    for c in range(S // CH):
        pltpu.make_async_copy(o_ref.at[pl.ds(c * CH, CH), 0:D], out_hbm.at[pl.ds(c * CH, CH), 0:D], osem.at[c]).wait()


KW = 29
VW = 7


@jax.jit
def pallas_concat_heads__sliding_block__ssm_conv_s4__prompt_kernel(
    A_x: jax.Array,
    A_wqkv: jax.Array,
    A_wo: jax.Array,
    B_u: jax.Array,
    B_A_re: jax.Array,
    B_A_im: jax.Array,
    B_B_re: jax.Array,
    B_B_im: jax.Array,
    B_C_re: jax.Array,
    B_C_im: jax.Array,
    B_log_dt: jax.Array,
    B_Dskip: jax.Array,
):
    out = pl.pallas_call(
        fused_kernel,
        out_shape=jax.ShapeDtypeStruct((S, 2 * D), bf16),
        in_specs=[pl.BlockSpec(memory_space=pl.ANY)] * 4 + [pl.BlockSpec(memory_space=pltpu.VMEM)] * 8,
        out_specs=pl.BlockSpec(memory_space=pl.ANY),
        scratch_shapes=[
            pltpu.VMEM((S, D), bf16),
            pltpu.VMEM((D, 3 * D), bf16),
            pltpu.VMEM((D, D), bf16),
            pltpu.VMEM((L, D), bf16),
            pltpu.VMEM((S, 2 * D), bf16),
            pltpu.SemaphoreType.DMA((3 + S // CH,)),
            pltpu.SemaphoreType.DMA((S // CH + 1,)),
            pltpu.VMEM((4, S, 128), bf16),
            pltpu.VMEM((4, S + W, 128), bf16),
            pltpu.VMEM((D, S + W), bf16),
            pltpu.VMEM((D, S), bf16),
            pltpu.VMEM((5, WIN, 128), f32),
            pltpu.VMEM((WIN, 16 * QB), f32),
            pltpu.VMEM((WIN, 16 * QB), f32),
            pltpu.VMEM((1, 16 * QB), f32),
            pltpu.VMEM((1, 16 * QB), f32),
            pltpu.VMEM((D, D), bf16),
            pltpu.VMEM((18, D, NM), f32),
            pltpu.VMEM((40 * 256, 128), f32),
            pltpu.VMEM((4 * L, 128), f32),
            pltpu.VMEM((32 * 128, 256), bf16),
            pltpu.VMEM((32, 256, 256), f32),
            pltpu.VMEM((32, 256, 256), f32),
            pltpu.VMEM((4 * L, 128), f32),
            pltpu.VMEM((64, 128), f32),
            pltpu.VMEM((32 * 256, 128), bf16),
        ],
        compiler_params=pltpu.CompilerParams(vmem_limit_bytes=110 * 1024 * 1024),
    )(A_x[0], A_wqkv, A_wo, B_u[0], B_A_re, B_A_im, B_B_re, B_B_im, B_C_re, B_C_im, B_log_dt, B_Dskip)
    return out[None]
```
